```python
import os as _os
_os.environ.setdefault('JAX_PLATFORMS', 'cpu')
import jax
import jax.numpy as jnp

def _softmax(x, axis=-1):
    return jax.nn.softmax(x, axis=axis)

def _gelu(x):
    return jax.nn.gelu(x, approximate=True)

def _silu(x):
    return jax.nn.silu(x)

def _sigmoid(x):
    return jax.nn.sigmoid(x)

def _layernorm(x, axis=-1, eps=1e-05):
    m = jnp.mean(x, axis=axis, keepdims=True)
    v = jnp.var(x, axis=axis, keepdims=True)
    return (x - m) / jnp.sqrt(v + eps)

def _scatter_add(tgt, idx, src, axis=0):
    return tgt.at[idx].add(src)

def _segment_sum(src, seg, n):
    return jax.ops.segment_sum(src, seg, n)

class _Rng:

    def __init__(self, key):
        self._k = key

    def _next(self):
        self._k, sub = jax.random.split(self._k)
        return sub

    def normal(self, shape):
        return jax.random.normal(self._next(), shape, dtype=jnp.bfloat16)

    def randint(self, lo, hi, shape):
        return jax.random.randint(self._next(), shape, lo, hi, dtype=jnp.int32)

    def uniform(self, shape, lo=0.0, hi=1.0):
        return jax.random.uniform(self._next(), shape, jnp.bfloat16, lo, hi)

    def permutation(self, n):
        return jax.random.permutation(self._next(), n)
kernel_name = 'gated_mix__sliding_block__memory_aug_recurrent_mem_tr__prompt'

def setup_inputs():
    _rng = _Rng(jax.random.key(int.from_bytes(__import__("os").urandom(4), "little")))
    _w = lambda a: (lambda t: t.astype(jnp.bfloat16) if jnp.issubdtype(t.dtype, jnp.floating) else t)(jnp.asarray(a))

    def _A_setup():
        B, S, D = (1, 2048, 448)
        return {'x': _w((lambda *s: _rng.normal(s) * 0.05)(B, S, D)), 'wqkv': _w((lambda *s: _rng.normal(s) * 0.8)(D, 3 * D)), 'wo': _w((lambda *s: _rng.normal(s) * 0.05)(D, D))}
    _A_in = _A_setup()

    def _B_setup():
        B, S, Dm = (1, 2048, 448)
        H, Dh = (16, 256)
        M, seg = (8, 32)
        seg = min(seg, S)
        S = S // seg * seg
        return {'x': _w((lambda *s: _rng.normal(s) * 0.05)(B, S, Dm)), 'mem0': _w((lambda *s: _rng.normal(s) * 0.8)(B, M, Dm)), 'Wq': _w((lambda *s: _rng.normal(s) * 3.2)(Dm, H, Dh) * Dm ** (-0.5)), 'Wk': _w((lambda *s: _rng.normal(s) * 3.2)(Dm, H, Dh) * Dm ** (-0.5)), 'Wv': _w((lambda *s: _rng.normal(s) * 0.8)(Dm, H, Dh) * Dm ** (-0.5)), 'Wo': _w((lambda *s: _rng.normal(s) * 0.8)(H, Dh, Dm) * (H * Dh) ** (-0.5)), 'seg_len': seg}
    _B_in = _B_setup()
    return {'A_x': _A_in['x'], 'A_wqkv': _A_in['wqkv'], 'A_wo': _A_in['wo'], 'B_x': _B_in['x'], 'B_mem0': _B_in['mem0'], 'B_Wq': _B_in['Wq'], 'B_Wk': _B_in['Wk'], 'B_Wv': _B_in['Wv'], 'B_Wo': _B_in['Wo'], 'B_seg_len': _B_in['seg_len'], 'gate_w': _w((lambda *s: _rng.normal(s) * 0.05)(448) * 16.0)}

def reference(A_x, A_wqkv, A_wo, B_x, B_mem0, B_Wq, B_Wk, B_Wv, B_Wo, B_seg_len, gate_w):

    def _A_ref(x, wqkv, wo):
        B, S, D = x.shape
        H = 16
        Dh = D // H
        W = 256
        qkv = (lambda x, *d: x.transpose(*d))((x @ wqkv).reshape(B, S, 3, H, Dh), 2, 0, 3, 1, 4)
        q, k, v = (qkv[0], qkv[1], qkv[2])
        scores = jnp.einsum('bhqd,bhkd->bhqk', q, k) * Dh ** (-0.5)
        idx = jnp.arange(S)
        mask = (idx[:, None] - idx[None, :] >= 0) & (idx[:, None] - idx[None, :] < W)
        scores = jnp.where(mask[None, None], scores, -1000000000.0)
        p = _softmax(scores, axis=-1)
        o = jnp.einsum('bhqk,bhkd->bhqd', p, v)
        return (lambda x, *d: x.transpose(*d))(o, 0, 2, 1, 3).reshape(B, S, D) @ wo

    def _B_ref(x, mem0, Wq, Wk, Wv, Wo, seg_len):
        B, S, Dm = x.shape
        H, Dh = (Wq.shape[1], Wq.shape[2])
        M = mem0.shape[1]
        scale = Dh ** (-0.5)
        n_seg = S // seg_len
        L = M + seg_len
        idx = jnp.arange(L)
        mask = (idx[:, None] < M) | (idx[:, None] >= idx[None, :])
        mem = mem0
        outs = []
        for s in range(n_seg):
            xs = x[:, s * seg_len:(s + 1) * seg_len, :].copy()
            h = jnp.concatenate([mem, xs], axis=1)
            q = jnp.einsum('btd,dhe->bhte', h, Wq)
            k = jnp.einsum('btd,dhe->bhte', h, Wk)
            v = jnp.einsum('btd,dhe->bhte', h, Wv)
            scores = jnp.einsum('bhqe,bhke->bhqk', q, k) * scale
            scores = jnp.where(mask[None, None], scores, -1000000000.0)
            p = _softmax(scores, axis=-1)
            o = jnp.einsum('bhqk,bhke->bhqe', p, v)
            o = jnp.einsum('bhte,hed->btd', o, Wo)
            mem = o[:, :M, :].copy()
            outs.append(o[:, M:, :])
        return jnp.concatenate(outs, axis=1)
    x = A_x
    g = _sigmoid((x * gate_w).sum(-1, keepdims=True))
    a = _A_ref(x, A_wqkv, A_wo)
    b = _B_ref(x, B_mem0, B_Wq, B_Wk, B_Wv, B_Wo, B_seg_len)
    return g * a + (1 - g) * b
```

```python
import functools

import jax
import jax.numpy as jnp
import jax.experimental.pallas as pl
import jax.experimental.pallas.tpu as pltpu

F32 = jnp.float32
BF16 = jnp.bfloat16
U32 = jnp.uint32

NT = (((1,), (1,)), ((), ()))
TN = (((0,), (0,)), ((), ()))

S = 2048
D = 448
H = 16
DHA = 28
DHB = 256
MEM = 8
SEG = 32
L = MEM + SEG
BLK = 128
NBLK = S // BLK
WIN = 256
NQT = H * DHB // 128
NUT = H * D // 128
NTILES = 2 * NQT + NUT
NQUART = NTILES // 4
NEG = -1e9
SCALE_A = 0.189453125
SCALE_B = 0.0625
MODE = "mix"


def _dot(a, b):
    return jnp.dot(a, b, preferred_element_type=F32)


def _dotg(a, b, dims):
    return jax.lax.dot_general(a, b, dims, preferred_element_type=F32)


def _merge(*streams):
    items = []
    for si, st in enumerate(streams):
        n = len(st)
        for k, t in enumerate(st):
            items.append(((k + 0.5) / n, si, k, t))
    items.sort(key=lambda x: (x[0], x[1], x[2]))
    return [t for _, _, _, t in items]


def _kernel(xat_h, wqkv_h, woa_h, mem0_h, wq_h, wk_h, wv_h, wot_h, gate_h,
            out_h,
            xat, wqkv, woa, gate, xb, mem, raw, wot, wbig,
            wka, wqvt, woat, ka, qt, vt, gsig, obuf, sbuf, pbuf, xp, bbuf, outb,
            sems, osem):
    cp = pltpu.make_async_copy

    c_wqkv = cp(wqkv_h, wqkv, sems.at[0])
    c_xa = cp(xat_h, xat, sems.at[1])
    c_wqkv.start()
    c_xa.start()
    c_woa = cp(woa_h, woa, sems.at[2])
    c_gate = cp(gate_h, gate, sems.at[3])
    c_wv = [cp(wv_h.at[:, pl.ds(128 * c, 128)], raw.at[0, c], sems.at[4 + c]) for c in range(2)]
    c_wo = cp(wot_h, wot, sems.at[6])
    c_wq = [cp(wq_h.at[:, pl.ds(128 * c, 128)], raw.at[1, c], sems.at[7 + c]) for c in range(2)]
    c_wk = [cp(wk_h.at[:, pl.ds(128 * c, 128)], raw.at[2, c], sems.at[9 + c]) for c in range(2)]
    c_mem = cp(mem0_h, mem, sems.at[12])
    c_wqkv.wait()
    c_xa.wait()
    for c in [c_woa, c_gate, c_mem] + c_wv + [c_wo] + c_wq + c_wk:
        c.start()

    for p in range(3):
        for g in range(4):
            col0 = p * D + 112 * g
            start = (col0 // 128) * 128
            width = min(256, 3 * D - start)
            win = wqkv[:, pl.ds(start, width)]
            if p == 1:
                ci = jax.lax.broadcasted_iota(jnp.int32, (width, 128), 0)
                ni = jax.lax.broadcasted_iota(jnp.int32, (width, 128), 1)
                src = col0 - start + DHA * (ni // 32) + ni % 32
                sel = jnp.where((ci == src) & (ni % 32 < DHA), 1.0, 0.0).astype(BF16)
                wka[g] = _dot(win, sel).astype(BF16)
            else:
                nit = jax.lax.broadcasted_iota(jnp.int32, (128, width), 0)
                cit = jax.lax.broadcasted_iota(jnp.int32, (128, width), 1)
                src = col0 - start + DHA * (nit // 32) + nit % 32
                selt = jnp.where((cit == src) & (nit % 32 < DHA), 1.0, 0.0).astype(BF16)
                row0 = (0 if p == 0 else 512) + 128 * g
                wqvt[pl.ds(row0, 128), :] = _dotg(selt, win, NT).astype(BF16)

    c_woa.wait()
    c_gate.wait()
    ri = jax.lax.broadcasted_iota(jnp.int32, (128, 112), 0)
    cj = jax.lax.broadcasted_iota(jnp.int32, (128, 112), 1)
    selo = jnp.where((cj == DHA * (ri // 32) + ri % 32) & (ri % 32 < DHA), 1.0, 0.0).astype(BF16)
    eye_r = jax.lax.broadcasted_iota(jnp.int32, (D, D), 0)
    eye_c = jax.lax.broadcasted_iota(jnp.int32, (D, D), 1)
    eye = jnp.where(eye_r == eye_c, 1.0, 0.0).astype(BF16)
    for g in range(4):
        wop = _dot(selo, woa[pl.ds(112 * g, 112), :]).astype(BF16)
        woat[:, pl.ds(128 * g, 128)] = _dotg(eye, wop, NT).astype(BF16)
    gate8 = jnp.broadcast_to(gate[...].reshape(1, D), (8, D))

    zk = jnp.zeros((WIN, 128), BF16)
    for g in range(4):
        ka[g, pl.ds(0, WIN), :] = zk
    for kb in range(2):
        vt[kb] = jnp.zeros((4, 128, 128), BF16)

    def a_proj(jb, carry):
        r0 = pl.multiple_of(jb * BLK, BLK)
        xt = xat[:, pl.ds(r0, BLK)]
        xblk = xt.T
        xb[pl.ds(r0, BLK), :] = xblk
        for g in range(4):
            ka[g, pl.ds(WIN + r0, BLK), :] = _dot(xblk, wka[g]).astype(BF16)
        for g in range(4):
            q = _dot(wqvt[pl.ds(128 * g, 128), :], xt)
            qt[jb, g] = (q * SCALE_A).astype(BF16)
            v = _dot(wqvt[pl.ds(512 + 128 * g, 128), :], xt)
            vt[jb + 2, g] = v.astype(BF16)
        gsig[jb] = jax.nn.sigmoid(_dot(gate8, xt))
        return carry

    jax.lax.fori_loop(0, NBLK, a_proj, 0)

    c_mem.wait()

    kr = jax.lax.broadcasted_iota(jnp.int32, (BLK, BLK), 0)
    qc = jax.lax.broadcasted_iota(jnp.int32, (BLK, BLK), 1)

    def a_attn_tasks(jb, slot, g):
        r0 = pl.multiple_of(jb * BLK, BLK)
        st = {}

        def scores():
            kwin = ka[g, pl.ds(r0, 3 * BLK), :]
            m0 = (kr > qc) & (jb >= 2)
            m1 = jb >= 1
            m2 = kr <= qc
            for hh in range(4):
                qs = qt[jb, g, pl.ds(32 * hh, 32), :]
                parts = []
                if hh > 0:
                    parts.append(jnp.zeros((32 * hh, BLK), BF16))
                parts.append(qs)
                if hh < 3:
                    parts.append(jnp.zeros((96 - 32 * hh, BLK), BF16))
                qm = jnp.concatenate(parts, axis=0)
                s = _dot(kwin, qm)
                s0 = jnp.where(m0, s[0:BLK], NEG)
                s1 = jnp.where(m1, s[BLK:2 * BLK], NEG)
                s2 = jnp.where(m2, s[2 * BLK:], NEG)
                st[hh] = jnp.max(jnp.maximum(jnp.maximum(s0, s1), s2), axis=0, keepdims=True)
                sbuf[hh, 0] = s0
                sbuf[hh, 1] = s1
                sbuf[hh, 2] = s2

        def expo(hh, kb):
            def f():
                e = jnp.exp(sbuf[hh, kb] - st[hh])
                part = jnp.sum(e, axis=0, keepdims=True)
                st[('l', hh)] = part if kb == 0 else st[('l', hh)] + part
                pbuf[hh, pl.ds(BLK * kb, BLK), :] = e.astype(BF16)
            return f

        def pv():
            for hh in range(4):
                vwin = jnp.concatenate(
                    [vt[jb + kb, g, pl.ds(32 * hh, 32), :] for kb in range(3)], axis=1)
                o = _dot(vwin, pbuf[hh]) / st[('l', hh)]
                obuf[slot, g, pl.ds(32 * hh, 32), :] = o.astype(BF16)

        return scores, [expo(hh, kb) for hh in range(4) for kb in range(3)], pv

    for g in range(4):
        a_sc, a_ex, a_pv = a_attn_tasks(0, 0, g)
        a_sc()
        for t in a_ex:
            t()
        a_pv()

    def relayout(src_idx, c, j):
        a = raw.bitcast(U32)[src_idx, c, pl.ds(j, D, stride=8), :]
        lo = pltpu.bitcast(a << 16, F32)
        hi = pltpu.bitcast(a & jnp.uint32(0xFFFF0000), F32)
        return lo, hi

    def put_w(n, val):
        wbig[n] = pltpu.bitcast(val.astype(BF16), U32)

    def get_w(n):
        return pltpu.bitcast(wbig[n], BF16)

    for c in c_wv:
        c.wait()
    c_wo.wait()
    z64 = jnp.zeros((64, DHB), BF16)
    for j in range(8):
        l0, h0 = relayout(0, 0, j)
        l1, h1 = relayout(0, 1, j)
        wv_e = jnp.concatenate([l0.astype(BF16), l1.astype(BF16)], axis=1)
        wv_o = jnp.concatenate([h0.astype(BF16), h1.astype(BF16)], axis=1)
        wo_e = jnp.concatenate([wot[pl.ds(2 * D * j, D), :], z64], axis=0)
        wo_o = jnp.concatenate([z64, wot[pl.ds(2 * D * j + D, D), :]], axis=0)
        be = _dotg(wv_e, wo_e, NT)
        bo = _dotg(wv_o, wo_o, NT)
        t0 = 2 * NQT + 7 * j
        for t in range(3):
            put_w(t0 + t, be[:, 128 * t:128 * (t + 1)])
        put_w(t0 + 3, be[:, 384:512] + bo[:, 0:128])
        for t in range(1, 4):
            put_w(t0 + 3 + t, bo[:, 128 * t:128 * (t + 1)])
    for c in c_wq:
        c.wait()
    for j in range(8):
        for c in range(2):
            lo, hi = relayout(1, c, j)
            put_w(4 * j + c, lo * SCALE_B)
            put_w(4 * j + 2 + c, hi * SCALE_B)
    for c in c_wk:
        c.wait()
    for j in range(8):
        for c in range(2):
            lo, hi = relayout(2, c, j)
            put_w(NQT + 4 * j + c, lo)
            put_w(NQT + 4 * j + 2 + c, hi)

    def xrow(r):
        return (r // SEG) * L + MEM + r % SEG

    def main_tasks(j, i, with_mem):
        nb = j + (i + 1) // 4
        ii = (i + 1) % 4
        src = pl.multiple_of(jnp.minimum(nb * BLK + 24 * ii, S - 24), 8)
        st = {}

        def prep():
            xr = xb[pl.ds(src, 24), :]
            st['lhs'] = jnp.concatenate([mem[...], xr], axis=0)

        def tile(n):
            def f():
                y = _dot(st['lhs'], get_w(n)).astype(BF16)
                if with_mem:
                    xp[n, j % 2, pl.ds(L * i, 8), :] = y[0:8]
                for t in range(3):
                    xp[n, nb % 2, pl.ds(xrow(24 * ii + 8 * t), 8), :] = y[8 + 8 * t:16 + 8 * t]
            return f
        return prep, tile

    def extra_tasks(j, i):
        nb = j + (i + 1) // 4
        ii = (i + 1) % 4
        src = pl.multiple_of(jnp.minimum(nb * BLK + 96, S - 32), 8)
        st = {}

        def tile(t):
            def f():
                if 'lhs' not in st:
                    st['lhs'] = xb[pl.ds(src, 32), :]
                n = ii * NQUART + t
                xp[n, nb % 2, pl.ds(xrow(96), 32), :] = _dot(st['lhs'], get_w(n)).astype(BF16)
            return f
        return [tile(t) for t in range(NQUART)]

    prep, tile = main_tasks(-1, 3, False)
    prep()
    for n in range(NTILES):
        tile(n)()
    for t in extra_tasks(-1, 3):
        t()

    ku = jax.lax.broadcasted_iota(jnp.int32, (L, L), 0)
    qq = jax.lax.broadcasted_iota(jnp.int32, (L, L), 1)
    bmask = (qq < MEM) | (qq >= ku)
    groups = [(0, 2, 4), (1, 3, 5), (6, 8, 10), (7, 9, 11), (12, 14), (13, 15)]

    def segment(j, i, atasks):
        st = {'acc': [None, None]}
        prep, mtile = main_tasks(j, i, True)

        def xt(n):
            return xp[n, j % 2, pl.ds(L * i, L), :]

        def b_scores(h):
            def f():
                q = jnp.concatenate([xt(2 * h), xt(2 * h + 1)], axis=1)
                k = jnp.concatenate([xt(NQT + 2 * h), xt(NQT + 2 * h + 1)], axis=1)
                st[h] = _dotg(k, q, NT)
            return f

        def b_softmax(h):
            def f():
                s = jnp.where(bmask, st[h], NEG)
                mx = jnp.max(s, axis=0, keepdims=True)
                e = jnp.exp(s - mx)
                l = jnp.sum(e, axis=0, keepdims=True)
                st[h] = (e / l).astype(BF16)
            return f

        def b_pv(grp):
            def f():
                par = grp[0] % 2
                p = jnp.concatenate([st[h] for h in grp], axis=0)
                u = jnp.concatenate(
                    [jnp.concatenate([xt(2 * NQT + (7 * h) // 2 + t) for t in range(4)], axis=1)
                     for h in grp], axis=0)
                o = _dotg(p, u, TN)
                st['acc'][par] = o if st['acc'][par] is None else st['acc'][par] + o
            return f

        def fin():
            a0, a1 = st['acc']
            o = a0 + jnp.concatenate([a1[:, 64:512], jnp.zeros((L, 64), F32)], axis=1)
            ob = o.astype(BF16)
            mem[...] = ob[0:MEM, :D]
            bbuf[j % 2, pl.ds(SEG * i, SEG), :] = ob[MEM:]

        a_sc, a_ex, a_pv, pre, post = atasks
        prep()
        for t in pre:
            t()
        for hp in range(H // 2):
            for h in (2 * hp, 2 * hp + 1):
                for n in (2 * h, 2 * h + 1, NQT + 2 * h, NQT + 2 * h + 1):
                    mtile(n)()
            if hp == 0:
                a_sc()
            if hp >= 1:
                b_scores(2 * hp - 2)()
                b_scores(2 * hp - 1)()
            if hp >= 2:
                b_softmax(2 * hp - 4)()
                b_softmax(2 * hp - 3)()
            if 1 <= hp <= 6:
                a_ex[2 * hp - 2]()
                a_ex[2 * hp - 1]()
        ready_after = {g: 2 * NQT + (7 * max(g)) // 2 + 3 + 4 for g in groups}
        pend = list(groups)
        for n in range(2 * NQT, NTILES):
            mtile(n)()
            if n == 2 * NQT + 3:
                b_scores(H - 2)()
                b_scores(H - 1)()
                b_softmax(H - 4)()
                b_softmax(H - 3)()
            if n == 2 * NQT + 8:
                b_softmax(H - 2)()
                b_softmax(H - 1)()
                a_pv()
            while pend and ready_after[pend[0]] <= n:
                b_pv(pend.pop(0))()
        ex = extra_tasks(j, i)
        k = 0
        for g in pend:
            for _ in range(6):
                ex[k]()
                k += 1
            b_pv(g)()
        for _ in range(8):
            ex[k]()
            k += 1
        fin()
        for t in ex[k:]:
            t()
        for t in post:
            t()

    def mix_tasks(jb, slot):
        st = {}

        def amm():
            ot = obuf[slot].reshape(512, BLK)
            st['a'] = _dot(woat[...], ot)

        def btr():
            st['b'] = bbuf[slot].T[:D].astype(F32)

        def out():
            g = gsig[jb][0:1]
            if MODE == 'a':
                res = st['a']
            elif MODE == 'b':
                res = st['b']
            else:
                res = g * st['a'] + (1.0 - g) * st['b']
            dst = out_h.at[:, pl.ds(pl.multiple_of(jb * BLK, BLK), BLK)]
            cp(outb, dst, osem).wait()
            outb[...] = res.astype(BF16)
            cp(outb, dst, osem).start()
        return amm, btr, out

    bbuf[1] = jnp.zeros((BLK, 512), BF16)
    obuf[1] = jnp.zeros((4, 128, BLK), BF16)
    outb[...] = jnp.zeros((D, BLK), BF16)
    cp(outb, out_h.at[:, pl.ds(0, BLK)], osem).start()

    def block(j, carry):
        jp = jnp.maximum(j - 1, 0)
        amm, btr, out = mix_tasks(jp, (j + 1) % 2)
        jn = jnp.minimum(j + 1, NBLK - 1)
        for i in range(4):
            a_sc, a_ex, a_pv = a_attn_tasks(jn, (j + 1) % 2, i)
            pre = [amm, btr] if i == 0 else []
            post = [out] if i == 3 else []
            segment(j, i, (a_sc, a_ex, a_pv, pre, post))
        return carry

    jax.lax.fori_loop(0, NBLK, block, 0)

    amm, btr, out = mix_tasks(NBLK - 1, (NBLK - 1) % 2)
    amm()
    btr()
    out()
    cp(outb, out_h.at[:, pl.ds(0, BLK)], osem).wait()


@functools.partial(jax.jit, static_argnames=("B_seg_len",))
def pallas_gated_mix__sliding_block__memory_aug_recurrent_mem_tr__prompt_kernel(A_x, A_wqkv, A_wo, B_x, B_mem0, B_Wq, B_Wk, B_Wv, B_Wo, B_seg_len, gate_w):
    assert B_seg_len == SEG
    hbm = pl.BlockSpec(memory_space=pltpu.HBM)
    scratch = [
        pltpu.VMEM((D, S), BF16),
        pltpu.VMEM((D, 3 * D), BF16),
        pltpu.VMEM((D, D), BF16),
        pltpu.VMEM((D,), BF16),
        pltpu.VMEM((S, D), BF16),
        pltpu.VMEM((MEM, D), BF16),
        pltpu.VMEM((3, 2, D * H, 128), BF16),
        pltpu.VMEM((H * D, DHB), BF16),
        pltpu.VMEM((NTILES, D // 2, 128), U32),
        pltpu.VMEM((4, D, 128), BF16),
        pltpu.VMEM((1024, D), BF16),
        pltpu.VMEM((D, 512), BF16),
        pltpu.VMEM((4, S + WIN, 128), BF16),
        pltpu.VMEM((NBLK, 4, 128, 128), BF16),
        pltpu.VMEM((NBLK + 2, 4, 128, 128), BF16),
        pltpu.VMEM((NBLK, 8, 128), F32),
        pltpu.VMEM((2, 4, 128, 128), BF16),
        pltpu.VMEM((4, 3, 128, 128), F32),
        pltpu.VMEM((4, 3 * BLK, 128), BF16),
        pltpu.VMEM((NTILES, 2, 4 * L, 128), BF16),
        pltpu.VMEM((2, BLK, 512), BF16),
        pltpu.VMEM((D, BLK), BF16),
        pltpu.SemaphoreType.DMA((13,)),
        pltpu.SemaphoreType.DMA(()),
    ]
    out_t = pl.pallas_call(
        _kernel,
        out_shape=jax.ShapeDtypeStruct((D, S), BF16),
        in_specs=[hbm] * 9,
        out_specs=hbm,
        scratch_shapes=scratch,
        compiler_params=pltpu.CompilerParams(vmem_limit_bytes=100 * 1024 * 1024),
    )(
        A_x.reshape(S, D).T, A_wqkv, A_wo, B_mem0.reshape(MEM, D),
        B_Wq.reshape(D * H, DHB), B_Wk.reshape(D * H, DHB), B_Wv.reshape(D * H, DHB),
        jnp.transpose(B_Wo, (0, 2, 1)).reshape(H * D, DHB), gate_w,
    )
    return out_t.T.reshape(1, S, D)
```

```python
import functools

import jax
import jax.numpy as jnp
import jax.experimental.pallas as pl
import jax.experimental.pallas.tpu as pltpu

F32 = jnp.float32
BF16 = jnp.bfloat16
U32 = jnp.uint32

NT = (((1,), (1,)), ((), ()))
TN = (((0,), (0,)), ((), ()))

S = 2048
D = 448
H = 16
DHA = 28
DHB = 256
MEM = 8
SEG = 32
L = MEM + SEG
BLK = 128
NBLK = S // BLK
WIN = 256
NQT = H * DHB // 128
NUT = H * D // 128
NTILES = 2 * NQT + NUT
NQUART = NTILES // 4
NEG = -1e9
SCALE_A = 0.189453125
SCALE_B = 0.0625
MODE = "mix"


def _dot(a, b):
    return jnp.dot(a, b, preferred_element_type=F32)


def _dotg(a, b, dims):
    return jax.lax.dot_general(a, b, dims, preferred_element_type=F32)


def _merge(*streams):
    items = []
    for si, st in enumerate(streams):
        n = len(st)
        for k, t in enumerate(st):
            items.append(((k + 0.5) / n, si, k, t))
    items.sort(key=lambda x: (x[0], x[1], x[2]))
    return [t for _, _, _, t in items]


def _kernel(xat_h, wqkv_h, woa_h, mem0_h, wq_h, wk_h, wv_h, wot_h, gate_h,
            out_h,
            xat, wqkv, woa, gate, xb, mem, raw, wot, wbig, wvl, shared,
            wka, wqvt, woat, ka, qt, vt, gsig, obuf, sbuf, pbuf, xp, ptb, bbuf, outb,
            zsm, sems, osem):
    cp = pltpu.make_async_copy
    zsm[0] = 0

    c_wqkv = cp(wqkv_h, wqkv, sems.at[0])
    c_xa = [cp(xat_h.at[:, pl.ds(512 * c, 512)], xat.at[:, pl.ds(512 * c, 512)], sems.at[13 + c])
            for c in range(4)]
    c_woa = cp(woa_h, woa, sems.at[2])
    c_gate = cp(gate_h, gate, sems.at[3])
    c_wv = [cp(wv_h.at[:, pl.ds(128 * c, 128)], raw.at[0, c], sems.at[4 + c]) for c in range(2)]
    c_wo = cp(wot_h, wot, sems.at[6])
    c_wq = [cp(wq_h.at[:, pl.ds(128 * c, 128)], raw.at[1, c], sems.at[7 + c]) for c in range(2)]
    c_wk = [cp(wk_h.at[:, pl.ds(128 * c, 128)], raw.at[2, c], sems.at[9 + c]) for c in range(2)]
    c_mem = cp(mem0_h, mem, sems.at[12])
    c_wqkv.start()
    c_gate.start()
    c_xa[0].start()
    c_woa.start()
    c_wqkv.wait()
    for c in c_xa[1:] + [c_mem] + c_wv + [c_wo] + c_wq + c_wk:
        c.start()

    nrow = jax.lax.broadcasted_iota(jnp.int32, (1, 128), 1)
    trow = jnp.where(nrow % 32 < DHA, DHA * (nrow // 32) + nrow % 32, -4096)
    ncol = jax.lax.broadcasted_iota(jnp.int32, (128, 1), 0)
    tcol = jnp.where(ncol % 32 < DHA, DHA * (ncol // 32) + ncol % 32, -4096)
    for p in (0, 2, 1):
        for g in range(4):
            col0 = p * D + 112 * g
            start = (col0 // 128) * 128
            width = min(256, 3 * D - start)
            win = wqkv[:, pl.ds(start, width)]
            if p == 1:
                ci = jax.lax.broadcasted_iota(jnp.int32, (width, 128), 0)
                sel = jnp.where(ci == trow + (col0 - start), 1.0, 0.0).astype(BF16)
                wka[g] = _dot(win, sel).astype(BF16)
            else:
                cit = jax.lax.broadcasted_iota(jnp.int32, (128, width), 1)
                selt = jnp.where(cit == tcol + (col0 - start), 1.0, 0.0).astype(BF16)
                row0 = (0 if p == 0 else 512) + 128 * g
                wqvt[pl.ds(row0, 128), :] = _dotg(selt, win, NT).astype(BF16)

    c_gate.wait()
    gate8 = jnp.broadcast_to(gate[...].reshape(1, D), (8, D))

    lane = jax.lax.broadcasted_iota(jnp.int32, (WIN, 128), 1)
    zk = jnp.where(lane % 32 == DHA, NEG, 0.0).astype(BF16)
    for g in range(4):
        ka[g, pl.ds(0, WIN), :] = zk
    qpad = jax.lax.broadcasted_iota(jnp.int32, (128, BLK), 0) % 32 == DHA
    for kb in range(2):
        vt[kb] = jnp.zeros((4, 128, 128), BF16)

    def a_proj(jb, carry):
        r0 = pl.multiple_of(jb * BLK, BLK)
        xt = xat[:, pl.ds(r0, BLK)]
        xblk = xt.T
        xb[pl.ds(r0, BLK), :] = xblk
        for g in range(4):
            q = _dot(wqvt[pl.ds(128 * g, 128), :], xt)
            qt[jb, g] = jnp.where(qpad, 1.0, q * SCALE_A).astype(BF16)
            v = _dot(wqvt[pl.ds(512 + 128 * g, 128), :], xt)
            vt[jb + 2, g] = v.astype(BF16)
        gsig[jb] = jax.nn.sigmoid(_dot(gate8, xt))
        for g in range(4):
            ka[g, pl.ds(WIN + r0, BLK), :] = _dot(xblk, wka[g]).astype(BF16)
        return carry

    for c in range(4):
        c_xa[c].wait()
        jax.lax.fori_loop(4 * c, 4 * c + 4, a_proj, 0, unroll=2)

    c_woa.wait()
    cj = jax.lax.broadcasted_iota(jnp.int32, (128, 112), 1)
    selo = jnp.where(cj == tcol, 1.0, 0.0).astype(BF16)
    for g in range(4):
        wop = _dot(selo, woa[pl.ds(112 * g, 112), :]).astype(BF16)
        woat[:, pl.ds(128 * g, 128)] = wop.T
    c_mem.wait()

    kr = jax.lax.broadcasted_iota(jnp.int32, (BLK, BLK), 0)
    qc = jax.lax.broadcasted_iota(jnp.int32, (BLK, BLK), 1)

    def a_attn_tasks(jb, slot, g, sa=0, sb=0):
        r0 = pl.multiple_of(jb * BLK, BLK)
        st = {}

        def scores():
            kwin = ka[g, pl.ds(r0, 3 * BLK), :]
            for hh in range(4):
                qs = qt[jb, g, pl.ds(32 * hh, 32), :]
                parts = []
                if hh > 0:
                    parts.append(jnp.zeros((32 * hh, BLK), BF16))
                parts.append(qs)
                if hh < 3:
                    parts.append(jnp.zeros((96 - 32 * hh, BLK), BF16))
                qm = jnp.concatenate(parts, axis=0)
                s = _dot(kwin, qm)
                s0 = jnp.where(kr > qc, s[0:BLK], NEG)
                s1 = s[BLK:2 * BLK]
                s2 = jnp.where(kr <= qc, s[2 * BLK:], NEG)
                st[hh] = jnp.max(jnp.maximum(jnp.maximum(s0, s1), s2), axis=0, keepdims=True)
                sbuf[sa, hh, pl.ds(0, BLK), :] = s0
                sbuf[sa, hh, pl.ds(BLK, BLK), :] = s1
                sbuf[sa, hh, pl.ds(2 * BLK, BLK), :] = s2

        def expo(hh, c):
            def f(gate=None):
                mx = st[hh] if gate is None else st[hh] + gate()
                e = jnp.exp(sbuf[sb, hh, pl.ds(96 * c, 96), :] - mx)
                part = jnp.sum(e, axis=0, keepdims=True)
                st[('l', hh)] = part if c == 0 else st[('l', hh)] + part
                pbuf[hh, pl.ds(96 * c, 96), :] = e.astype(BF16)
            return f

        def pv():
            for hh in range(4):
                vwin = jnp.concatenate(
                    [vt[jb + kb, g, pl.ds(32 * hh, 32), :] for kb in range(3)], axis=1)
                o = _dot(vwin, pbuf[hh]) / st[('l', hh)]
                obuf[slot, g, pl.ds(32 * hh, 32), :] = o.astype(BF16)

        return scores, [expo(hh, c) for hh in range(4) for c in range(4)], pv

    raw32 = raw.bitcast(U32)
    RC = 112

    def relayout(src_idx, c, j, r):
        a = raw32[src_idx, c, pl.ds(j + 8 * RC * r, RC, stride=8), :]
        lo = pltpu.bitcast(a << 16, F32)
        hi = pltpu.bitcast(a & jnp.uint32(0xFFFF0000), F32)
        return lo.astype(BF16), hi.astype(BF16)

    def put_w(n, val, r=None):
        if r is None:
            wbig[n] = pltpu.bitcast(val, U32)
        else:
            wbig[n, pl.ds(RC // 2 * r, RC // 2), :] = pltpu.bitcast(val, U32)

    def get_w(n):
        return pltpu.bitcast(wbig[n], BF16)

    z64 = jnp.zeros((64, DHB), BF16)

    def fold_prep(j):
        for c in range(2):
            for r in range(D // RC):
                lo, hi = relayout(0, c, j, r)
                wvl[j % 2, 0, pl.ds(RC * r, RC), pl.ds(128 * c, 128)] = lo
                wvl[j % 2, 1, pl.ds(RC * r, RC), pl.ds(128 * c, 128)] = hi

    def fold_mm(j, odd):
        wv = wvl[j % 2, odd]
        w = wot[pl.ds(2 * D * j + D * odd, D), :]
        t0 = 2 * NQT + 7 * j
        if not odd:
            be = _dotg(wv, jnp.concatenate([w, z64], axis=0), NT)
            for t in range(3):
                put_w(t0 + t, be[:, 128 * t:128 * (t + 1)].astype(BF16))
            shared[...] = be[:, 384:512]
        else:
            bo = _dotg(wv, jnp.concatenate([z64, w], axis=0), NT)
            put_w(t0 + 3, (shared[...] + bo[:, 0:128]).astype(BF16))
            for t in range(1, 4):
                put_w(t0 + 3 + t, bo[:, 128 * t:128 * (t + 1)].astype(BF16))

    def relay_qk(which, j, c):
        base = 0 if which == 1 else NQT
        for r in range(D // RC):
            lo, hi = relayout(which, c, j, r)
            put_w(base + 4 * j + c, lo, r)
            put_w(base + 4 * j + 2 + c, hi, r)

    def xrow(r):
        return (r // SEG) * L + MEM + r % SEG

    def main_tasks(j, i, with_mem, with_x=True):
        nb = j + (i + 1) // 4
        ii = (i + 1) % 4
        src = pl.multiple_of(jnp.minimum(nb * BLK + 24 * ii, S - 24), 8)
        st = {}

        def prep():
            if with_x:
                xr = xb[pl.ds(src, 24), :]
                st['lhs'] = jnp.concatenate([mem[...], xr], axis=0)
            else:
                st['lhs'] = mem[...]

        def tile(n):
            def f():
                y32 = _dot(st['lhs'], get_w(n))
                st['last'] = y32[0:1]
                y = y32.astype(BF16)
                if with_mem:
                    xp[n, j % 2, pl.ds(L * i, 8), :] = y[0:8]
                if with_x:
                    for t in range(3):
                        xp[n, nb % 2, pl.ds(xrow(24 * ii + 8 * t), 8), :] = y[8 + 8 * t:16 + 8 * t]
            return f

        def gate():
            bits = pltpu.bitcast(st['last'], jnp.int32) & zsm[0]
            return pltpu.bitcast(bits, F32)
        return prep, tile, gate

    def extra_tasks(j, i):
        nb = j + (i + 1) // 4
        ii = (i + 1) % 4
        src = pl.multiple_of(jnp.minimum(nb * BLK + 96, S - 32), 8)
        st = {}

        def tile(t):
            def f():
                if 'lhs' not in st:
                    st['lhs'] = xb[pl.ds(src, 32), :]
                n = ii * NQUART + t
                xp[n, nb % 2, pl.ds(xrow(96), 32), :] = _dot(st['lhs'], get_w(n)).astype(BF16)
            return f
        return [tile(t) for t in range(NQUART)]

    prep, tile, _ = main_tasks(-1, 3, False)
    ex0 = extra_tasks(-1, 3)
    a0 = []
    for g in range(4):
        a_sc, a_ex, a_pv = a_attn_tasks(0, 0, g)
        a0.append([a_sc] + a_ex + [a_pv])
    for c in c_wv:
        c.wait()
    fold_prep(0)
    c_wo.wait()
    prep()
    for j in range(8):
        fold_mm(j, 0)
        if j < 7:
            fold_prep(j + 1)
        if j == 0:
            for c in c_wq:
                c.wait()
        if j == 4:
            for c in c_wk:
                c.wait()
        which, jj0 = (1, 2 * j) if j < 4 else (2, 2 * (j - 4))
        for c in range(2):
            relay_qk(which, jj0, c)
        fold_mm(j, 1)
        for c in range(2):
            relay_qk(which, jj0 + 1, c)
        if j < 4:
            for t in a0[j]:
                t()
        else:
            for n in range(8 * (j - 4), 8 * (j - 4) + 8):
                tile(n)()
        if j >= 1:
            for n in range(2 * NQT + 7 * (j - 1), 2 * NQT + 7 * j):
                tile(n)()
    for t in ex0:
        t()
    for n in range(2 * NQT + 49, NTILES):
        tile(n)()
    for n in range(NQT, 2 * NQT):
        tile(n)()

    ku = jax.lax.broadcasted_iota(jnp.int32, (L, L), 0)
    qq = jax.lax.broadcasted_iota(jnp.int32, (L, L), 1)
    bmask = (qq < MEM) | (qq >= ku)
    groups = [(0, 2, 4), (1, 3, 5), (6, 8, 10), (7, 9, 11), (12, 14), (13, 15)]

    def segment(j, i, atasks, last=False):
        st = {'acc': [None, None]}
        ptslot_w = j % 2
        ptslot_r = 1 - (j + 1) % 2
        tail = last and i == 3
        prep, mtile, gate = main_tasks(j, i, True, not tail)

        def xt(n):
            return xp[n, j % 2, pl.ds(L * i, L), :]

        def rows_qk(base, grp):
            return jnp.concatenate(
                [jnp.concatenate([xt(base + 2 * h), xt(base + 2 * h + 1)], axis=1) for h in grp], axis=0)

        def b_scores(grp):
            def f():
                st[grp] = _dotg(rows_qk(NQT, grp), rows_qk(0, grp), NT) * SCALE_B
            return f

        def b_softmax(grp):
            def f():
                n = len(grp)
                row = jax.lax.broadcasted_iota(jnp.int32, (L, L * n), 0)
                lane = jax.lax.broadcasted_iota(jnp.int32, (L, L * n), 1)
                blocks = []
                for a in range(n):
                    t = lane - L * a
                    inblk = (t >= 0) & (t < L)
                    s = jnp.where(inblk & ((t < MEM) | (t >= row)), st[grp][L * a:L * (a + 1)], NEG)
                    mx = jnp.max(s, axis=0, keepdims=True)
                    e = jnp.exp(s - mx)
                    l = jnp.sum(e, axis=0, keepdims=True)
                    blocks.append(e * jnp.where(inblk[0:1], 1.0 / l, 0.0))
                blocks.append(jnp.zeros((128 - L * n, L * n), F32))
                p = jnp.concatenate(blocks, axis=0)
                p = jnp.concatenate([p, jnp.zeros((128, 128 - L * n), F32)], axis=1).T
                lhs = p[0:L]
                for a in range(1, n):
                    lhs = lhs + p[L * a:L * (a + 1)]
                lhs = jnp.concatenate([lhs, jnp.zeros((8, 128), F32)], axis=0)
                ptb[ptslot_w, groups.index(grp)] = lhs.astype(BF16)
            return f

        def b_pv(grp):
            def f():
                par = grp[0] % 2
                kk = L * len(grp)
                p = ptb[ptslot_r, groups.index(grp)][:L, :kk]
                u = jnp.concatenate(
                    [jnp.concatenate([xt(2 * NQT + (7 * h) // 2 + t) for t in range(4)], axis=1)
                     for h in grp], axis=0)
                o = _dot(p, u)
                st['acc'][par] = o if st['acc'][par] is None else st['acc'][par] + o
            return f

        def fin():
            a0, a1 = st['acc']
            o = a0 + jnp.concatenate([a1[:, 64:512], jnp.zeros((L, 64), F32)], axis=1)
            ob = o.astype(BF16)
            mem[...] = ob[0:MEM, :D]
            bbuf[j % 2, pl.ds(SEG * i, SEG), :] = ob[MEM:]

        a_sc, a_ex, a_pv, pre, post = atasks
        prep()
        for t in pre:
            t()
        nex = 0
        for h in range(H):
            for n in (2 * h, 2 * h + 1, NQT + 2 * h, NQT + 2 * h + 1):
                mtile(n)()
            if h >= 4:
                if not last:
                    a_ex[nex](gate)
                nex += 1
            if h == 1 and not last:
                a_sc()
            if h in (7, 13):
                gi = 0 if h == 7 else 2
                b_scores(groups[gi])()
                b_scores(groups[gi + 1])()
            if h in (9, 15):
                b_softmax(groups[0 if h == 9 else 2])()
            if h == 11:
                b_softmax(groups[1])()
        ready_after = {g: 2 * NQT + (7 * max(g)) // 2 + 3 + 6 for g in groups}
        pend = list(groups)
        for n in range(2 * NQT, NTILES):
            mtile(n)()
            if n == 2 * NQT + 3:
                b_softmax(groups[3])()
            if n == 2 * NQT + 5:
                b_scores(groups[4])()
                b_scores(groups[5])()
            if n == 2 * NQT + 12:
                b_softmax(groups[4])()
            if n == 2 * NQT + 18:
                b_softmax(groups[5])()
            if n % 4 == 1 and nex < 16:
                if not last:
                    a_ex[nex](gate)
                nex += 1
            if n == 2 * NQT + 24 and not last:
                a_pv()
            while pend and ready_after[pend[0]] <= n:
                b_pv(pend.pop(0))()
        ex = [(lambda: None)] * NQUART if tail else extra_tasks(j, i)
        k = 0
        for g in pend:
            for _ in range(6):
                ex[k]()
                k += 1
            b_pv(g)()
        for _ in range(8):
            ex[k]()
            k += 1
        fin()
        for t in ex[k:]:
            t()
        for t in post:
            t()

    def mix_tasks(jb, slot):
        st = {}

        def amm():
            ot = obuf[slot].reshape(512, BLK)
            st['a'] = _dot(woat[...], ot)

        def btr():
            st['b'] = bbuf[slot].T[:D].astype(F32)

        def out():
            g = gsig[jb][0:1]
            if MODE == 'a':
                res = st['a']
            elif MODE == 'b':
                res = st['b']
            else:
                res = g * st['a'] + (1.0 - g) * st['b']
            dst = out_h.at[:, pl.ds(pl.multiple_of(jb * BLK, BLK), BLK)]
            cp(outb, dst, osem).wait()
            outb[...] = res.astype(BF16)
            cp(outb, dst, osem).start()
        return amm, btr, out

    bbuf[1] = jnp.zeros((BLK, 512), BF16)
    obuf[1] = jnp.zeros((4, 128, BLK), BF16)
    outb[...] = jnp.zeros((D, BLK), BF16)
    cp(outb, out_h.at[:, pl.ds(0, BLK)], osem).start()

    def block(j, carry, last=False):
        jp = jnp.maximum(j - 1, 0)
        amm, btr, out = mix_tasks(jp, (j + 1) % 2)
        jn = jnp.minimum(j + 1, NBLK - 1)
        for i in range(4):
            a_sc, a_ex, a_pv = a_attn_tasks(jn, (j + 1) % 2, i, j % 2, 1 - (j + 1) % 2)
            pre = [amm, btr] if i == 0 else []
            post = [out] if i == 3 else []
            segment(j, i, (a_sc, a_ex, a_pv, pre, post), last)
        return carry

    jax.lax.fori_loop(0, NBLK - 1, block, 0)
    block(NBLK - 1 + zsm[0], 0, last=True)

    amm, btr, out = mix_tasks(NBLK - 1, (NBLK - 1) % 2)
    amm()
    btr()
    out()
    cp(outb, out_h.at[:, pl.ds(0, BLK)], osem).wait()


@functools.partial(jax.jit, static_argnames=("B_seg_len",))
def pallas_gated_mix__sliding_block__memory_aug_recurrent_mem_tr__prompt_kernel(A_x, A_wqkv, A_wo, B_x, B_mem0, B_Wq, B_Wk, B_Wv, B_Wo, B_seg_len, gate_w):
    assert B_seg_len == SEG
    hbm = pl.BlockSpec(memory_space=pltpu.HBM)
    scratch = [
        pltpu.VMEM((D, S), BF16),
        pltpu.VMEM((D, 3 * D), BF16),
        pltpu.VMEM((D, D), BF16),
        pltpu.VMEM((D,), BF16),
        pltpu.VMEM((S + 8, D), BF16),
        pltpu.VMEM((MEM, D), BF16),
        pltpu.VMEM((3, 2, D * H, 128), BF16),
        pltpu.VMEM((H * D, DHB), BF16),
        pltpu.VMEM((NTILES, D // 2, 128), U32),
        pltpu.VMEM((2, 2, D, DHB), BF16),
        pltpu.VMEM((D, 128), F32),
        pltpu.VMEM((4, D, 128), BF16),
        pltpu.VMEM((1024, D), BF16),
        pltpu.VMEM((D, 512), BF16),
        pltpu.VMEM((4, S + WIN, 128), BF16),
        pltpu.VMEM((NBLK, 4, 128, 128), BF16),
        pltpu.VMEM((NBLK + 2, 4, 128, 128), BF16),
        pltpu.VMEM((NBLK, 8, 128), F32),
        pltpu.VMEM((2, 4, 128, 128), BF16),
        pltpu.VMEM((2, 4, 3 * BLK, 128), F32),
        pltpu.VMEM((4, 3 * BLK, 128), BF16),
        pltpu.VMEM((NTILES, 2, 4 * L, 128), BF16),
        pltpu.VMEM((2, 6, 48, 128), BF16),
        pltpu.VMEM((2, BLK, 512), BF16),
        pltpu.VMEM((D, BLK), BF16),
        pltpu.SMEM((1,), jnp.int32),
        pltpu.SemaphoreType.DMA((17,)),
        pltpu.SemaphoreType.DMA(()),
    ]
    out_t = pl.pallas_call(
        _kernel,
        out_shape=jax.ShapeDtypeStruct((D, S), BF16),
        in_specs=[hbm] * 9,
        out_specs=hbm,
        scratch_shapes=scratch,
        compiler_params=pltpu.CompilerParams(vmem_limit_bytes=100 * 1024 * 1024),
    )(
        A_x.reshape(S, D).T, A_wqkv, A_wo, B_mem0.reshape(MEM, D),
        B_Wq.reshape(D * H, DHB), B_Wk.reshape(D * H, DHB), B_Wv.reshape(D * H, DHB),
        jnp.transpose(B_Wo, (0, 2, 1)).reshape(H * D, DHB), gate_w,
    )
    return out_t.T.reshape(1, S, D)
```

```python
import functools

import jax
import jax.numpy as jnp
import jax.experimental.pallas as pl
import jax.experimental.pallas.tpu as pltpu

F32 = jnp.float32
BF16 = jnp.bfloat16
U32 = jnp.uint32

NT = (((1,), (1,)), ((), ()))

S = 2048
D = 448
H = 16
DHA = 28
DHB = 256
MEM = 8
SEG = 32
L = MEM + SEG
BLK = 128
NBLK = S // BLK
WIN = 256
NQT = H * DHB // 128
NUT = H * D // 128
NTILES = 2 * NQT + NUT
NQUART = NTILES // 4
RC = 112
NRC = D // RC
NEG = -1e9
SCALE_A = 0.189453125
SCALE_B = 0.0625
MODE = "mix"
GROUPS = [(0, 2, 4), (1, 3, 5), (6, 8, 10), (7, 9, 11), (12, 14), (13, 15)]


def _dot(a, b):
    return jnp.dot(a, b, preferred_element_type=F32)


def _dotg(a, b, dims):
    return jax.lax.dot_general(a, b, dims, preferred_element_type=F32)


def _kernel(xat_h, wqkv_h, woa_h, mem0_h, wq_h, wk_h, wv_h, wot_h, gate_h,
            out_h,
            xat, wqkv, woa, gate, xb, mem, raw, wot, wbig, shared,
            wka, wqvt, woat, ka, qt, vt, gsig, obuf, sbuf, pbuf, xp, ptb, bbuf, outb,
            zsm, sems, osem):
    cp = pltpu.make_async_copy
    zsm[0] = 0

    def zero_like_bits(v):
        return pltpu.bitcast(v, U32) & zsm[0].astype(U32)

    c_wqkv = cp(wqkv_h, wqkv, sems.at[0])
    c_xa = cp(xat_h, xat, sems.at[1])
    c_woa = cp(woa_h, woa, sems.at[2])
    c_gate = cp(gate_h, gate, sems.at[3])
    c_mem = cp(mem0_h, mem, sems.at[4])
    c_wo = cp(wot_h, wot, sems.at[5])

    def c_w(m, src):
        return [cp(src.at[pl.ds(H * RC * r, H * RC), pl.ds(128 * c, 128)], raw.at[m, c, r], sems.at[6 + m])
                for c in range(2) for r in range(NRC)]

    c_wv, c_wq, c_wk = c_w(0, wv_h), c_w(1, wq_h), c_w(2, wk_h)
    c_wqkv.start()
    c_wqkv.wait()
    for c in [c_xa, c_gate, c_woa, c_mem]:
        c.start()

    nrow = jax.lax.broadcasted_iota(jnp.int32, (1, 128), 1)
    trow = jnp.where(nrow % 32 < DHA, DHA * (nrow // 32) + nrow % 32, -4096)
    ncol = jax.lax.broadcasted_iota(jnp.int32, (128, 1), 0)
    tcol = jnp.where(ncol % 32 < DHA, DHA * (ncol // 32) + ncol % 32, -4096)
    for p in (0, 2, 1):
        for g in range(4):
            col0 = p * D + 112 * g
            start = (col0 // 128) * 128
            width = min(256, 3 * D - start)
            win = wqkv[:, pl.ds(start, width)]
            if p == 1:
                ci = jax.lax.broadcasted_iota(jnp.int32, (width, 128), 0)
                sel = jnp.where(ci == trow + (col0 - start), 1.0, 0.0).astype(BF16)
                wka[g] = _dot(win, sel).astype(BF16)
            else:
                cit = jax.lax.broadcasted_iota(jnp.int32, (128, width), 1)
                selt = jnp.where(cit == tcol + (col0 - start), 1.0, 0.0).astype(BF16)
                row0 = (0 if p == 0 else 512) + 128 * g
                wqvt[pl.ds(row0 // 2, 64), :] = pltpu.bitcast(_dotg(selt, win, NT).astype(BF16), U32)

    lane = jax.lax.broadcasted_iota(jnp.int32, (WIN, 128), 1)
    zk = jnp.where(lane % 32 == DHA, NEG, 0.0).astype(BF16)
    for g in range(4):
        ka[g, pl.ds(0, WIN), :] = zk
    for kb in range(2):
        vt[kb] = jnp.zeros((4, 128, 128), BF16)
    c_gate.wait()
    c_woa.wait()
    cj = jax.lax.broadcasted_iota(jnp.int32, (128, 112), 1)
    selo = jnp.where(cj == tcol, 1.0, 0.0).astype(BF16)
    for g in range(4):
        wop = _dot(selo, woa[pl.ds(112 * g, 112), :]).astype(BF16)
        woat[:, pl.ds(128 * g, 128)] = wop.T

    def gated(lhs, zbits):
        if zbits is None:
            return lhs
        head = pltpu.bitcast(pltpu.bitcast(lhs[0:16, 0:128], U32) | zbits, BF16)
        top = jnp.concatenate([head, lhs[0:16, 128:]], axis=1)
        return jnp.concatenate([top, lhs[16:]], axis=0)

    def a_proj_tasks(jb):
        r0 = pl.multiple_of(jb * BLK, BLK)
        st = {}

        def tr():
            xb[pl.ds(r0, BLK), :] = xat[:, pl.ds(r0, BLK)].T

        def qv(k):
            def f(zbits):
                lhs = gated(pltpu.bitcast(wqvt[pl.ds(128 * k, 128), :], BF16), zbits)
                y = _dot(lhs, xat[:, pl.ds(r0, BLK)])
                st['last'] = y[0:1]
                st['probe'] = [y[64 * c:64 * c + 1] for c in range(4)]
                for gg in range(2):
                    g = (2 * k + gg) % 4
                    yg = y[128 * gg:128 * (gg + 1)]
                    if k < 2:
                        qpad = jax.lax.broadcasted_iota(jnp.int32, (128, BLK), 0) % 32 == DHA
                        qt[jb, g] = jnp.where(qpad, 1.0, yg * SCALE_A).astype(BF16)
                    else:
                        vt[jb + 2, g] = yg.astype(BF16)
            return f

        def kk(k):
            def f(zbits):
                if k == 0:
                    gate8 = jnp.broadcast_to(gate[...].reshape(1, D), (8, D))
                    gsig[jb] = jax.nn.sigmoid(_dot(gate8, xat[:, pl.ds(r0, BLK)]))
                xblk = gated(xb[pl.ds(r0, BLK), :], zbits)
                for g in (2 * k, 2 * k + 1):
                    y = _dot(xblk, wka[g])
                    st['last'] = y[0:1]
                    st['probe'] = [y[32 * c:32 * c + 1] for c in range(4)]
                    ka[g, pl.ds(WIN + r0, BLK), :] = y.astype(BF16)
            return f

        def gate_fn(c=None):
            v = st['last'] if c is None else st['probe'][c]
            return pltpu.bitcast(zero_like_bits(v), F32)

        return tr, [qv(0), qv(1), qv(2), qv(3), kk(0), kk(1)], gate_fn

    def a_attn_tasks(jb, slot, g, sa=0, sb=0, kbs=(0, 1, 2)):
        r0 = pl.multiple_of(jb * BLK + BLK * kbs[0], BLK)
        nk = BLK * len(kbs)
        ch = nk // 4
        st = {}

        def scores():
            kr = jax.lax.broadcasted_iota(jnp.int32, (BLK, BLK), 0)
            qc = jax.lax.broadcasted_iota(jnp.int32, (BLK, BLK), 1)
            kwin = ka[g, pl.ds(r0, nk), :]
            for hh in range(4):
                qs = qt[jb, g, pl.ds(32 * hh, 32), :]
                parts = []
                if hh > 0:
                    parts.append(jnp.zeros((32 * hh, BLK), BF16))
                parts.append(qs)
                if hh < 3:
                    parts.append(jnp.zeros((96 - 32 * hh, BLK), BF16))
                qm = jnp.concatenate(parts, axis=0)
                s = _dot(kwin, qm)
                mx = None
                for x, kb in enumerate(kbs):
                    sk = s[BLK * x:BLK * (x + 1)]
                    if kb == 0:
                        sk = jnp.where(kr > qc, sk, NEG)
                    elif kb == 2:
                        sk = jnp.where(kr <= qc, sk, NEG)
                    mx = sk if mx is None else jnp.maximum(mx, sk)
                    sbuf[sa, hh, pl.ds(BLK * x, BLK), :] = sk
                st[hh] = jnp.max(mx, axis=0, keepdims=True)

        def expo(hh, c):
            def f(gate_fn):
                mx = st[hh] + gate_fn()
                e = jnp.exp(sbuf[sb, hh, pl.ds(ch * c, ch), :] - mx)
                part = jnp.sum(e, axis=0, keepdims=True)
                st[('l', hh)] = part if c == 0 else st[('l', hh)] + part
                pbuf[hh, pl.ds(ch * c, ch), :] = e.astype(BF16)
            return f

        def pv():
            for hh in range(4):
                vwin = jnp.concatenate(
                    [vt[jb + kb, g, pl.ds(32 * hh, 32), :] for kb in kbs], axis=1)
                o = _dot(vwin, pbuf[hh, pl.ds(0, nk), :]) / st[('l', hh)]
                obuf[slot, g, pl.ds(32 * hh, 32), :] = o.astype(BF16)

        return scores, [expo(hh, c) for hh in range(4) for c in range(4)], pv

    raw32 = raw.bitcast(U32)

    def get_w(n):
        return pltpu.bitcast(wbig[n], BF16)

    def put_w(n, val):
        wbig[n] = pltpu.bitcast(val.astype(BF16), U32)

    def relay_chunk(m, base, r, j, c, zf=None):
        a = raw32[m, c, r, pl.ds(j, RC, stride=8), :]
        if zf is not None:
            a = a | zf
        lo = pltpu.bitcast(a << 16, F32).astype(BF16)
        hi = pltpu.bitcast(a & jnp.uint32(0xFFFF0000), F32).astype(BF16)
        lo, hi = pltpu.bitcast(lo, U32), pltpu.bitcast(hi, U32)
        rows = pl.ds(pl.multiple_of(RC // 2 * r, 8), RC // 2)
        wbig[base + 4 * j + c, rows, :] = lo
        wbig[base + 4 * j + 2 + c, rows, :] = hi
        return lo[RC // 2 - 8:] | hi[RC // 2 - 8:]

    def a_proj_loop(lo, hi, m, with_attn, pre=None):
        def body(jb, carry):
            if pre is not None:
                pre(jb)
            tr, stages, gate_fn = a_proj_tasks(jb)
            jc = [(j, c) for j in range(8) for c in range(2)]
            split = [0, 4, 8, 12, 16, 16, 16]
            asplit = [0, 3, 6, 9, 12, 16, 16]
            if with_attn:
                a_sc, a_ex, a_pv = a_attn_tasks(0, 0, jb % 4, jb // 16, (jb + 16) // 32 , kbs=(2,))
            tr()
            if with_attn:
                a_sc()
            due = [None] * 8
            for k, stage in enumerate(stages):
                zin = due[k]
                if k > 0:
                    chain = pltpu.bitcast(gate_fn(), U32)
                    chain = jnp.broadcast_to(chain, (8, 128))
                    zin = chain if zin is None else zin | chain
                stage(zin)
                z = None
                if m is not None:
                    mm, base = m(jb)
                    for ci, (j, c) in enumerate(jc[split[k]:split[k + 1]]):
                        zz = relay_chunk(mm, base, jb % NRC, j, c, pltpu.bitcast(gate_fn(ci % 4), U32))
                        z = zz if z is None else z | zz
                    if z is not None:
                        due[min(k + 2, 5)] = (z & zsm[0].astype(U32)) if due[min(k + 2, 5)] is None else (z & zsm[0].astype(U32)) | due[min(k + 2, 5)]
                if with_attn and k < 5:
                    for t in a_ex[asplit[k]:asplit[k + 1]]:
                        t(gate_fn)
            if with_attn:
                a_pv()
            return carry
        jax.lax.fori_loop(lo, hi, body, 0)

    def starter(at, copies):
        def pre(jb):
            @pl.when(jb == at)
            def _():
                for c in copies:
                    c.start()
        return pre

    c_xa.wait()
    for c in c_wv:
        c.start()
    a_proj_loop(0, 8, None, False, starter(4, c_wq))
    for c in c_wv:
        c.wait()
    a_proj_loop(8, 12, lambda jb: (0, NTILES), True, starter(8, [c_wo]))
    for c in c_wq:
        c.wait()
    a_proj_loop(12, 16, lambda jb: (1, 0), False, starter(12, c_wk))

    def xrow(r):
        return (r // SEG) * L + MEM + r % SEG

    def main_tasks(j, i, with_mem, with_x=True):
        nb = j + (i + 1) // 4
        ii = (i + 1) % 4
        src = pl.multiple_of(jnp.minimum(nb * BLK + 24 * ii, S - 24), 8)
        st = {}

        def prep():
            if with_x:
                xr = xb[pl.ds(src, 24), :]
                st['lhs'] = jnp.concatenate([mem[...], xr], axis=0)
            else:
                st['lhs'] = mem[...]

        def tile(n):
            def f():
                y32 = _dot(st['lhs'], get_w(n))
                st['last'] = y32[0:1]
                y = y32.astype(BF16)
                if with_mem:
                    xp[n, j % 2, pl.ds(L * i, 8), :] = y[0:8]
                if with_x:
                    for t in range(3):
                        xp[n, nb % 2, pl.ds(xrow(24 * ii + 8 * t), 8), :] = y[8 + 8 * t:16 + 8 * t]
            return f

        def gate_fn():
            return pltpu.bitcast(zero_like_bits(st['last']), F32)
        return prep, tile, gate_fn

    def extra_tasks(j, i):
        nb = j + (i + 1) // 4
        ii = (i + 1) % 4
        src = pl.multiple_of(jnp.minimum(nb * BLK + 96, S - 32), 8)
        st = {}

        def tile(t):
            def f():
                if 'lhs' not in st:
                    st['lhs'] = xb[pl.ds(src, 32), :]
                n = ii * NQUART + t
                xp[n, nb % 2, pl.ds(xrow(96), 32), :] = _dot(st['lhs'], get_w(n)).astype(BF16)
            return f
        return tile

    c_mem.wait()
    c_wo.wait()
    z64 = jnp.zeros((64, DHB), BF16)

    prep0, tile0, _ = main_tasks(-1, 3, False)
    ex0 = extra_tasks(-1, 3)

    def fold_mm(h, half):
        j, odd = h // 2, h % 2
        t0 = 2 * NQT + 7 * j
        w = wot[pl.ds(D * h, D), :]
        w = jnp.concatenate([z64, w] if odd else [w, z64], axis=0)[256 * half:256 * half + 256]
        wv = jnp.concatenate([get_w(NTILES + 2 * h), get_w(NTILES + 2 * h + 1)], axis=1)
        b = _dotg(wv, w, NT)
        if not odd:
            put_w(t0 + 2 * half, b[:, 0:128])
            if half == 0:
                put_w(t0 + 1, b[:, 128:256])
            else:
                shared[...] = b[:, 128:256]
        else:
            if half == 0:
                put_w(t0 + 3, shared[...] + b[:, 0:128])
            else:
                put_w(t0 + 5, b[:, 0:128])
            put_w(t0 + 4 + 2 * half, b[:, 128:256])
        return [zero_like_bits(b[112 * c:112 * c + 1, 0:128]) for c in range(4)]

    prep0()
    kch = [(j, c, r) for j in range(8) for c in range(2) for r in range(NRC)]
    nk = 0
    for j in range(8):
        if j == 2:
            for c in c_wk:
                c.wait()
        for h in (2 * j, 2 * j + 1):
            for half in range(2):
                probes = fold_mm(h, half)
                if j >= 2:
                    for pz in probes[:3]:
                        if nk < len(kch):
                            jj, c, r = kch[nk]
                            relay_chunk(2, NQT, r, jj, c, pz)
                            nk += 1
        for n in range(4 * j, 4 * j + 4):
            tile0(n)()
        for t in range(4 * j, min(4 * j + 4, NQUART)):
            ex0(t)()
        if j >= 1:
            for n in range(2 * NQT + 7 * (j - 1), 2 * NQT + 7 * j):
                tile0(n)()
    assert nk == len(kch)
    for n in range(2 * NQT + 49, NTILES):
        tile0(n)()
    for n in range(NQT, 2 * NQT):
        tile0(n)()

    def segment(j, i, atasks, last=False):
        st = {'acc': [None, None]}
        ptslot_w = j % 2
        ptslot_r = 1 - (j + 1) % 2
        tail = last and i == 3
        prep, mtile, gate_fn = main_tasks(j, i, True, not tail)

        def xt(n):
            return xp[n, j % 2, pl.ds(L * i, L), :]

        def rows_qk(base, grp):
            return jnp.concatenate(
                [jnp.concatenate([xt(base + 2 * h), xt(base + 2 * h + 1)], axis=1) for h in grp], axis=0)

        def b_scores(grp):
            st[grp] = _dotg(rows_qk(NQT, grp), rows_qk(0, grp), NT) * SCALE_B

        def b_softmax(grp):
            n = len(grp)
            row = jax.lax.broadcasted_iota(jnp.int32, (L, L * n), 0)
            lane = jax.lax.broadcasted_iota(jnp.int32, (L, L * n), 1)
            blocks = []
            for a in range(n):
                t = lane - L * a
                inblk = (t >= 0) & (t < L)
                s = jnp.where(inblk & ((t < MEM) | (t >= row)), st[grp][L * a:L * (a + 1)], NEG)
                mx = jnp.max(s, axis=0, keepdims=True)
                e = jnp.exp(s - mx)
                l = jnp.sum(e, axis=0, keepdims=True)
                blocks.append(e * jnp.where(inblk[0:1], 1.0 / l, 0.0))
            blocks.append(jnp.zeros((128 - L * n, L * n), F32))
            p = jnp.concatenate(blocks, axis=0)
            p = jnp.concatenate([p, jnp.zeros((128, 128 - L * n), F32)], axis=1).T
            lhs = p[0:L]
            for a in range(1, n):
                lhs = lhs + p[L * a:L * (a + 1)]
            lhs = jnp.concatenate([lhs, jnp.zeros((8, 128), F32)], axis=0)
            ptb[ptslot_w, GROUPS.index(grp)] = lhs.astype(BF16)

        def b_pv(grp):
            par = grp[0] % 2
            kk = L * len(grp)
            p = ptb[ptslot_r, GROUPS.index(grp)][:L, :kk]
            u = jnp.concatenate(
                [jnp.concatenate([xt(2 * NQT + (7 * h) // 2 + t) for t in range(4)], axis=1)
                 for h in grp], axis=0)
            o = _dot(p, u)
            st['acc'][par] = o if st['acc'][par] is None else st['acc'][par] + o

        def fin():
            a0, a1 = st['acc']
            o = a0 + jnp.concatenate([a1[:, 64:512], jnp.zeros((L, 64), F32)], axis=1)
            ob = o.astype(BF16)
            if not tail:
                mem[...] = ob[0:MEM, :D]
            bbuf[j % 2, pl.ds(SEG * i, SEG), :] = ob[MEM:]

        a_sc, a_ex, a_pv, pre, post = atasks
        prep()
        for t in pre:
            t()
        nex = 0
        for h in range(H):
            for n in (2 * h, 2 * h + 1, NQT + 2 * h, NQT + 2 * h + 1):
                if tail and n < NQT:
                    continue
                mtile(n)()
            if h >= 4:
                if not last:
                    a_ex[nex](gate_fn)
                nex += 1
            if h == 1 and not last:
                a_sc()
            if h in (7, 13):
                gi = 0 if h == 7 else 2
                b_scores(GROUPS[gi])
                b_scores(GROUPS[gi + 1])
            if h in (9, 15):
                b_softmax(GROUPS[0 if h == 9 else 2])
            if h == 11:
                b_softmax(GROUPS[1])
        ready_after = {g: 2 * NQT + (7 * max(g)) // 2 + 3 + 6 for g in GROUPS}
        pend = list(GROUPS)
        for n in range(2 * NQT, NTILES):
            mtile(n)()
            if n == 2 * NQT + 3:
                b_softmax(GROUPS[3])
            if n == 2 * NQT + 5:
                b_scores(GROUPS[4])
                b_scores(GROUPS[5])
            if n == 2 * NQT + 12:
                b_softmax(GROUPS[4])
            if n == 2 * NQT + 18:
                b_softmax(GROUPS[5])
            if n % 4 == 1 and nex < 16:
                if not last:
                    a_ex[nex](gate_fn)
                nex += 1
            if n == 2 * NQT + 24 and not last:
                a_pv()
            while pend and ready_after[pend[0]] <= n:
                b_pv(pend.pop(0))
        ex = (lambda t: (lambda: None)) if tail else extra_tasks(j, i)
        k = 0
        for g in pend:
            for _ in range(6):
                ex(k)()
                k += 1
            b_pv(g)
        for _ in range(8):
            ex(k)()
            k += 1
        fin()
        while k < NQUART:
            ex(k)()
            k += 1
        for t in post:
            t()

    def mix_tasks(jb, slot):
        st = {}

        def amm():
            ot = obuf[slot].reshape(512, BLK)
            st['a'] = _dot(woat[...], ot)

        def btr():
            st['b'] = bbuf[slot].T[:D].astype(F32)

        def out():
            g = gsig[jb][0:1]
            if MODE == 'a':
                res = st['a']
            elif MODE == 'b':
                res = st['b']
            else:
                res = g * st['a'] + (1.0 - g) * st['b']
            dst = out_h.at[:, pl.ds(pl.multiple_of(jb * BLK, BLK), BLK)]
            cp(outb, dst, osem).wait()
            outb[...] = res.astype(BF16)
            cp(outb, dst, osem).start()
        return amm, btr, out

    bbuf[1] = jnp.zeros((BLK, 512), BF16)
    obuf[1] = jnp.zeros((4, 128, BLK), BF16)
    outb[...] = jnp.zeros((D, BLK), BF16)
    cp(outb, out_h.at[:, pl.ds(0, BLK)], osem).start()

    def block(j, carry, last=False):
        jp = jnp.maximum(j - 1, 0)
        amm, btr, out = mix_tasks(jp, (j + 1) % 2)
        jn = jnp.minimum(j + 1, NBLK - 1)
        amm2, btr2, out2 = mix_tasks(j, j % 2)
        for i in range(4):
            a_sc, a_ex, a_pv = a_attn_tasks(jn, (j + 1) % 2, i, j % 2, 1 - (j + 1) % 2)
            pre = [amm, btr] if i == 0 else []
            post = [out] if i == 3 else []
            if last:
                post = {0: [], 1: [out], 2: [amm2], 3: [btr2, out2]}[i]
            segment(j, i, (a_sc, a_ex, a_pv, pre, post), last)
        return carry

    jax.lax.fori_loop(0, NBLK - 1, block, 0)
    block(NBLK - 1 + zsm[0], 0, last=True)
    cp(outb, out_h.at[:, pl.ds(0, BLK)], osem).wait()


@functools.partial(jax.jit, static_argnames=("B_seg_len",))
def pallas_gated_mix__sliding_block__memory_aug_recurrent_mem_tr__prompt_kernel(A_x, A_wqkv, A_wo, B_x, B_mem0, B_Wq, B_Wk, B_Wv, B_Wo, B_seg_len, gate_w):
    assert B_seg_len == SEG
    hbm = pl.BlockSpec(memory_space=pltpu.HBM)
    scratch = [
        pltpu.VMEM((D, S), BF16),
        pltpu.VMEM((D, 3 * D), BF16),
        pltpu.VMEM((D, D), BF16),
        pltpu.VMEM((D,), BF16),
        pltpu.VMEM((S + 8, D), BF16),
        pltpu.VMEM((MEM, D), BF16),
        pltpu.VMEM((3, 2, NRC, H * RC, 128), BF16),
        pltpu.VMEM((H * D, DHB), BF16),
        pltpu.VMEM((NTILES + 2 * H, D // 2, 128), U32),
        pltpu.VMEM((D, 128), F32),
        pltpu.VMEM((4, D, 128), BF16),
        pltpu.VMEM((512, D), U32),
        pltpu.VMEM((D, 512), BF16),
        pltpu.VMEM((4, S + WIN, 128), BF16),
        pltpu.VMEM((NBLK, 4, 128, 128), BF16),
        pltpu.VMEM((NBLK + 2, 4, 128, 128), BF16),
        pltpu.VMEM((NBLK, 8, 128), F32),
        pltpu.VMEM((2, 4, 128, 128), BF16),
        pltpu.VMEM((2, 4, 3 * BLK, 128), F32),
        pltpu.VMEM((4, 3 * BLK, 128), BF16),
        pltpu.VMEM((NTILES, 2, 4 * L, 128), BF16),
        pltpu.VMEM((2, 6, 48, 128), BF16),
        pltpu.VMEM((2, BLK, 512), BF16),
        pltpu.VMEM((D, BLK), BF16),
        pltpu.SMEM((1,), jnp.int32),
        pltpu.SemaphoreType.DMA((9,)),
        pltpu.SemaphoreType.DMA(()),
    ]
    out_t = pl.pallas_call(
        _kernel,
        out_shape=jax.ShapeDtypeStruct((D, S), BF16),
        in_specs=[hbm] * 9,
        out_specs=hbm,
        scratch_shapes=scratch,
        compiler_params=pltpu.CompilerParams(vmem_limit_bytes=100 * 1024 * 1024),
    )(
        A_x.reshape(S, D).T, A_wqkv, A_wo, B_mem0.reshape(MEM, D),
        B_Wq.reshape(D * H, DHB), B_Wk.reshape(D * H, DHB), B_Wv.reshape(D * H, DHB),
        jnp.transpose(B_Wo, (0, 2, 1)).reshape(H * D, DHB), gate_w,
    )
    return out_t.T.reshape(1, S, D)
```

```python
import functools

import jax
import jax.numpy as jnp
import jax.experimental.pallas as pl
import jax.experimental.pallas.tpu as pltpu

F32 = jnp.float32
BF16 = jnp.bfloat16
U32 = jnp.uint32

NT = (((1,), (1,)), ((), ()))

S = 2048
D = 448
H = 16
DHA = 28
DHB = 256
MEM = 8
SEG = 32
L = MEM + SEG
BLK = 128
NBLK = S // BLK
WIN = 256
NHT = H * DHB // 128
NFT = H * D // 128
NTILES = 2 * NFT
NQUART = NTILES // 4
RC = 112
NRC = D // RC
NEG = -1e9
SCALE_A = 0.189453125
SCALE_B = 0.0625
GROUPS = [(0, 2, 4), (1, 3, 5), (6, 8, 10), (7, 9, 11), (12, 14), (13, 15)]


def _dot(a, b):
    return jnp.dot(a, b, preferred_element_type=F32)


def _dotg(a, b, dims):
    return jax.lax.dot_general(a, b, dims, preferred_element_type=F32)


def _kernel(xat_h, wqkv_h, woa_h, mem0_h, wq_h, wk_h, wv_h, wot_h, gate_h,
            out_h,
            xat, wqkv, woa, gate, xb, mem, raw, wot, wbig, wsq, wsk, wsv, shared,
            wka, wqvt, woat, ka, qt, vt, gsig, obuf, sbuf, pbuf, xp, ptb, bbuf, outb,
            zsm, sems, osem):
    cp = pltpu.make_async_copy
    zsm[0] = 0

    def zero_like_bits(v):
        return pltpu.bitcast(v, U32) & zsm[0].astype(U32)

    c_wqkv = cp(wqkv_h, wqkv, sems.at[0])
    c_xa = cp(xat_h, xat, sems.at[1])
    c_woa = cp(woa_h, woa, sems.at[2])
    c_gate = cp(gate_h, gate, sems.at[3])
    c_mem = cp(mem0_h, mem, sems.at[4])
    c_wo = cp(wot_h, wot, sems.at[5])

    def c_w(m, src):
        return [cp(src.at[pl.ds(H * RC * r, H * RC), pl.ds(128 * c, 128)], raw.at[m, c, r], sems.at[6 + m])
                for c in range(2) for r in range(NRC)]

    c_wv, c_wq, c_wk = c_w(0, wv_h), c_w(1, wq_h), c_w(2, wk_h)
    c_wqkv.start()
    c_wqkv.wait()
    for c in [c_xa, c_gate, c_woa, c_mem]:
        c.start()

    nrow = jax.lax.broadcasted_iota(jnp.int32, (1, 128), 1)
    trow = jnp.where(nrow % 32 < DHA, DHA * (nrow // 32) + nrow % 32, -4096)
    ncol = jax.lax.broadcasted_iota(jnp.int32, (128, 1), 0)
    tcol = jnp.where(ncol % 32 < DHA, DHA * (ncol // 32) + ncol % 32, -4096)
    for p in (0, 2, 1):
        for g in range(4):
            col0 = p * D + 112 * g
            start = (col0 // 128) * 128
            width = min(256, 3 * D - start)
            win = wqkv[:, pl.ds(start, width)]
            if p == 1:
                ci = jax.lax.broadcasted_iota(jnp.int32, (width, 128), 0)
                sel = jnp.where(ci == trow + (col0 - start), 1.0, 0.0).astype(BF16)
                wka[g] = _dot(win, sel).astype(BF16)
            else:
                cit = jax.lax.broadcasted_iota(jnp.int32, (128, width), 1)
                selt = jnp.where(cit == tcol + (col0 - start), 1.0, 0.0).astype(BF16)
                row0 = (0 if p == 0 else 512) + 128 * g
                wqvt[pl.ds(row0 // 2, 64), :] = pltpu.bitcast(_dotg(selt, win, NT).astype(BF16), U32)

    lane = jax.lax.broadcasted_iota(jnp.int32, (WIN, 128), 1)
    zk = jnp.where(lane % 32 == DHA, NEG, 0.0).astype(BF16)
    for g in range(4):
        ka[g, pl.ds(0, WIN), :] = zk
    for kb in range(2):
        vt[kb] = jnp.zeros((4, 128, 128), BF16)
    c_gate.wait()
    c_woa.wait()
    cj = jax.lax.broadcasted_iota(jnp.int32, (128, 112), 1)
    selo = jnp.where(cj == tcol, 1.0, 0.0).astype(BF16)
    for g in range(4):
        wop = _dot(selo, woa[pl.ds(112 * g, 112), :]).astype(BF16)
        woat[:, pl.ds(128 * g, 128)] = wop.T

    def gated(lhs, zbits):
        if zbits is None:
            return lhs
        head = pltpu.bitcast(pltpu.bitcast(lhs[0:16, 0:128], U32) | zbits, BF16)
        top = jnp.concatenate([head, lhs[0:16, 128:]], axis=1)
        return jnp.concatenate([top, lhs[16:]], axis=0)

    def a_proj_tasks(jb):
        r0 = pl.multiple_of(jb * BLK, BLK)
        st = {}

        def tr():
            xb[pl.ds(r0, BLK), :] = xat[:, pl.ds(r0, BLK)].T

        def qv(k):
            def f(zbits):
                lhs = gated(pltpu.bitcast(wqvt[pl.ds(128 * k, 128), :], BF16), zbits)
                y = _dot(lhs, xat[:, pl.ds(r0, BLK)])
                st['last'] = y[0:1]
                st['probe'] = [y[64 * c:64 * c + 1] for c in range(4)]
                for gg in range(2):
                    g = (2 * k + gg) % 4
                    yg = y[128 * gg:128 * (gg + 1)]
                    if k < 2:
                        qpad = jax.lax.broadcasted_iota(jnp.int32, (128, BLK), 0) % 32 == DHA
                        qt[jb, g] = jnp.where(qpad, 1.0, yg * SCALE_A).astype(BF16)
                    else:
                        vt[jb + 2, g] = yg.astype(BF16)
            return f

        def kk(k):
            def f(zbits):
                if k == 0:
                    gate8 = jnp.broadcast_to(gate[...].reshape(1, D), (8, D))
                    gsig[jb] = jax.nn.sigmoid(_dot(gate8, xat[:, pl.ds(r0, BLK)]))
                xblk = gated(xb[pl.ds(r0, BLK), :], zbits)
                for g in (2 * k, 2 * k + 1):
                    y = _dot(xblk, wka[g])
                    st['last'] = y[0:1]
                    st['probe'] = [y[32 * c:32 * c + 1] for c in range(4)]
                    ka[g, pl.ds(WIN + r0, BLK), :] = y.astype(BF16)
            return f

        def gate_fn(c=None):
            v = st['last'] if c is None else st['probe'][c]
            return pltpu.bitcast(zero_like_bits(v), F32)

        return tr, [qv(0), qv(1), qv(2), qv(3), kk(0), kk(1)], gate_fn

    def a_attn_tasks(jb, slot, g, sa=0, sb=0, kbs=(0, 1, 2)):
        r0 = pl.multiple_of(jb * BLK + BLK * kbs[0], BLK)
        nk = BLK * len(kbs)
        ch = nk // 4
        st = {}

        def scores():
            kr = jax.lax.broadcasted_iota(jnp.int32, (BLK, BLK), 0)
            qc = jax.lax.broadcasted_iota(jnp.int32, (BLK, BLK), 1)
            kwin = ka[g, pl.ds(r0, nk), :]
            for hh in range(4):
                qs = qt[jb, g, pl.ds(32 * hh, 32), :]
                parts = []
                if hh > 0:
                    parts.append(jnp.zeros((32 * hh, BLK), BF16))
                parts.append(qs)
                if hh < 3:
                    parts.append(jnp.zeros((96 - 32 * hh, BLK), BF16))
                qm = jnp.concatenate(parts, axis=0)
                s = _dot(kwin, qm)
                mx = None
                for x, kb in enumerate(kbs):
                    sk = s[BLK * x:BLK * (x + 1)]
                    if kb == 0:
                        sk = jnp.where(kr > qc, sk, NEG)
                    elif kb == 2:
                        sk = jnp.where(kr <= qc, sk, NEG)
                    mx = sk if mx is None else jnp.maximum(mx, sk)
                    sbuf[sa, hh, pl.ds(BLK * x, BLK), :] = sk
                st[hh] = jnp.max(mx, axis=0, keepdims=True)

        def expo(hh, c):
            def f(gate_fn):
                mx = st[hh] + gate_fn()
                e = jnp.exp(sbuf[sb, hh, pl.ds(ch * c, ch), :] - mx)
                part = jnp.sum(e, axis=0, keepdims=True)
                st[('l', hh)] = part if c == 0 else st[('l', hh)] + part
                pbuf[hh, pl.ds(ch * c, ch), :] = e.astype(BF16)
            return f

        def pv():
            for hh in range(4):
                vwin = jnp.concatenate(
                    [vt[jb + kb, g, pl.ds(32 * hh, 32), :] for kb in kbs], axis=1)
                o = _dot(vwin, pbuf[hh, pl.ds(0, nk), :]) / st[('l', hh)]
                obuf[slot, g, pl.ds(32 * hh, 32), :] = o.astype(BF16)

        return scores, [expo(hh, c) for hh in range(4) for c in range(4)], pv

    raw32 = raw.bitcast(U32)

    def get_w(n):
        return pltpu.bitcast(wbig[n], BF16)

    def put_w(n, val):
        wbig[n] = pltpu.bitcast(val.astype(BF16), U32)

    def relay_chunk(m, dst, r, j, c, zf=None):
        a = raw32[m, c, r, pl.ds(j, RC, stride=8), :]
        if zf is not None:
            a = a | zf
        lo = pltpu.bitcast(a << 16, F32).astype(BF16)
        hi = pltpu.bitcast(a & jnp.uint32(0xFFFF0000), F32).astype(BF16)
        lo, hi = pltpu.bitcast(lo, U32), pltpu.bitcast(hi, U32)
        rows = pl.ds(pl.multiple_of(RC // 2 * r, 8), RC // 2)
        dst[4 * j + c, rows, :] = lo
        dst[4 * j + 2 + c, rows, :] = hi
        return lo[RC // 2 - 8:] | hi[RC // 2 - 8:]

    def a_proj_loop(lo, hi, m, with_attn, pre=None):
        def body(jb, carry):
            if pre is not None:
                pre(jb)
            tr, stages, gate_fn = a_proj_tasks(jb)
            jc = [(j, c) for j in range(8) for c in range(2)]
            split = [0, 4, 8, 12, 16, 16, 16]
            asplit = [0, 3, 6, 9, 12, 16, 16]
            if with_attn:
                a_sc, a_ex, a_pv = a_attn_tasks(0, 0, jb % 4, jb // 16, (jb + 16) // 32, kbs=(2,))
            tr()
            if with_attn:
                a_sc()
            due = [None] * 8
            for k, stage in enumerate(stages):
                zin = due[k]
                if k > 0:
                    chain = pltpu.bitcast(gate_fn(), U32)
                    chain = jnp.broadcast_to(chain, (8, 128))
                    zin = chain if zin is None else zin | chain
                stage(zin)
                z = None
                if m is not None:
                    mm, dst = m
                    for ci, (j, c) in enumerate(jc[split[k]:split[k + 1]]):
                        zz = relay_chunk(mm, dst, jb % NRC, j, c, pltpu.bitcast(gate_fn(ci % 4), U32))
                        z = zz if z is None else z | zz
                    if z is not None:
                        due[k + 2] = z & zsm[0].astype(U32)
                if with_attn and k < 5:
                    for t in a_ex[asplit[k]:asplit[k + 1]]:
                        t(gate_fn)
            if with_attn:
                a_pv()
            return carry
        jax.lax.fori_loop(lo, hi, body, 0)

    def starter(at, copies):
        def pre(jb):
            @pl.when(jb == at)
            def _():
                for c in copies:
                    c.start()
        return pre

    c_xa.wait()
    for c in c_wv:
        c.start()
    a_proj_loop(0, 8, None, False, starter(4, c_wq))
    c_wo.start()
    for c in c_wv:
        c.wait()
    a_proj_loop(8, 12, (0, wsv), True, starter(10, c_wk))
    for c in c_wq:
        c.wait()
    a_proj_loop(12, 16, (1, wsq), False)

    def xrow(r):
        return (r // SEG) * L + MEM + r % SEG

    def main_tasks(j, i, with_mem):
        nb = j + (i + 1) // 4
        ii = (i + 1) % 4
        src = pl.multiple_of(jnp.minimum(nb * BLK + 24 * ii, S - 24), 8)
        st = {}

        def prep():
            xr = xb[pl.ds(src, 24), :]
            st['lhs'] = jnp.concatenate([mem[...], xr], axis=0)

        def tile(n):
            def f():
                y32 = _dot(st['lhs'], get_w(n))
                st['last'] = y32[0:1]
                y = y32.astype(BF16)
                if with_mem:
                    xp[n, j % 2, pl.ds(L * i, 8), :] = y[0:8]
                for t in range(3):
                    xp[n, nb % 2, pl.ds(xrow(24 * ii + 8 * t), 8), :] = y[8 + 8 * t:16 + 8 * t]
            return f

        def gate_fn():
            return pltpu.bitcast(zero_like_bits(st['last']), F32)
        return prep, tile, gate_fn, (lambda: st['lhs'][0:MEM])

    def extra_tasks(j, i):
        nb = j + (i + 1) // 4
        ii = (i + 1) % 4
        src = pl.multiple_of(jnp.minimum(nb * BLK + 96, S - 32), 8)
        st = {}

        def tile(t):
            def f():
                if 'lhs' not in st:
                    st['lhs'] = xb[pl.ds(src, 32), :]
                n = ii * NQUART + t
                xp[n, nb % 2, pl.ds(xrow(96), 32), :] = _dot(st['lhs'], get_w(n)).astype(BF16)
            return f
        return tile

    c_mem.wait()
    c_wo.wait()
    z64 = jnp.zeros((64, DHB), BF16)

    def head_w(src, h):
        return jnp.concatenate([pltpu.bitcast(src[2 * h], BF16), pltpu.bitcast(src[2 * h + 1], BF16)], axis=1)

    def fold_mm(kind, j, odd, half):
        h = 2 * j + odd
        if kind == 0:
            t0, lhs, w = 7 * j, head_w(wsq, h), head_w(wsk, h)
        else:
            t0, lhs, w = NFT + 7 * j, head_w(wsv, h), wot[pl.ds(pl.multiple_of(D * h, 64), D), :]
        w = jnp.concatenate([z64, w] if odd else [w, z64], axis=0)[256 * half:256 * half + 256]
        b = _dotg(lhs, w, NT)
        if kind == 0:
            b = b * SCALE_B
        if not odd:
            put_w(t0 + 2 * half, b[:, 0:128])
            if half == 0:
                put_w(t0 + 1, b[:, 128:256])
            else:
                shared[...] = b[:, 128:256]
        else:
            if half == 0:
                put_w(t0 + 3, shared[...] + b[:, 0:128])
            else:
                put_w(t0 + 5, b[:, 0:128])
            put_w(t0 + 4 + 2 * half, b[:, 128:256])
        return [zero_like_bits(b[112 * c:112 * c + 1, 0:128]) for c in range(4)]

    for c in c_wk:
        c.wait()

    def u_fold(r, carry):
        kch = [(jj, c) for jj in range(8) for c in range(2)]
        nk = 0
        for jp in range(2):
            for odd in range(2):
                for half in range(2):
                    probes = fold_mm(1, 2 * r + jp, odd, half)
                    for pz in probes[1:3]:
                        relay_chunk(2, wsk, r, kch[nk][0], kch[nk][1], pz)
                        nk += 1
        return carry

    jax.lax.fori_loop(0, NRC, u_fold, 0)

    def t_fold(j, carry):
        prep0, tile0, _, _ = main_tasks(-1, 3, False)
        ex0 = extra_tasks(-1, 3)
        prep0()
        for odd in range(2):
            for half in range(2):
                fold_mm(0, j, odd, half)
        for t in range(7):
            tile0(NFT + 7 * j + t)()
        for t in range(4):
            ex0(jnp.minimum(4 * j + t, NQUART - 1))()
        for t in range(7):
            tile0(7 * j + t)()
        return carry

    jax.lax.fori_loop(0, 8, t_fold, 0)

    def segment(j, i, atasks):
        st = {'acc': [None, None]}
        ptslot_w = j % 2
        ptslot_r = 1 - (j + 1) % 2
        prep, mtile, gate_fn, mem0_val = main_tasks(j, i, True)

        def xt(n):
            return xp[n, j % 2, pl.ds(L * i, L), :]

        def window(base, h):
            return jnp.concatenate([xt(base + (7 * h) // 2 + t) for t in range(4)], axis=1)

        def b_scores(grp):
            if 'hp' not in st:
                r = pl.multiple_of((4 * j + i) * SEG, SEG)
                hrows = jnp.concatenate([mem0_val(), xb[pl.ds(r, SEG), :]], axis=0)
                z = jnp.zeros((L, 64), BF16)
                st['hp'] = [jnp.concatenate([hrows, z], axis=1), jnp.concatenate([z, hrows], axis=1)]
            t = jnp.concatenate([window(0, h) for h in grp], axis=0)
            st[grp] = _dotg(st['hp'][grp[0] % 2], t, NT)

        def b_softmax(grp):
            n = len(grp)
            row = jax.lax.broadcasted_iota(jnp.int32, (L, L * n), 0)
            lane = jax.lax.broadcasted_iota(jnp.int32, (L, L * n), 1)
            blk = [(lane >= L * a) & (lane < L * (a + 1)) for a in range(n)]
            t = lane
            for a in range(1, n):
                t = jnp.where(lane >= L * a, lane - L * a, t)
            s = jnp.where((t < MEM) | (t >= row), st[grp], NEG)
            mx = jnp.max(s, axis=0, keepdims=True)
            e = jnp.exp(s - mx)
            l = jnp.sum(e, axis=0, keepdims=True)
            p = e * (1.0 / l)
            blocks = [jnp.where(blk[a], p, 0.0) for a in range(n)]
            blocks.append(jnp.zeros((128 - L * n, L * n), F32))
            p = jnp.concatenate(blocks, axis=0)
            p = jnp.concatenate([p, jnp.zeros((128, 128 - L * n), F32)], axis=1).T
            lhs = p[0:L]
            for a in range(1, n):
                lhs = lhs + p[L * a:L * (a + 1)]
            lhs = jnp.concatenate([lhs, jnp.zeros((8, 128), F32)], axis=0)
            ptb[ptslot_w, GROUPS.index(grp)] = lhs.astype(BF16)

        def b_pv(grp):
            par = grp[0] % 2
            kk = L * len(grp)
            p = ptb[ptslot_r, GROUPS.index(grp)][:L, :kk]
            u = jnp.concatenate([window(NFT, h) for h in grp], axis=0)
            o = _dot(p, u)
            st['acc'][par] = o if st['acc'][par] is None else st['acc'][par] + o

        def fin():
            a0, a1 = st['acc']
            o = a0 + jnp.concatenate([a1[:, 64:512], jnp.zeros((L, 64), F32)], axis=1)
            ob = o.astype(BF16)
            mem[...] = ob[0:MEM, :D]
            bbuf[j % 2, pl.ds(SEG * i, SEG), :] = ob[MEM:]

        a_sc, a_ex, a_pv, pre, post = atasks
        prep()
        for t in pre:
            t()
        nex = 0
        ready_after = {g: NFT + (7 * max(g)) // 2 + 3 + 6 for g in GROUPS}
        pend = list(GROUPS)
        for n in range(NTILES):
            mtile(n)()
            if n == 6:
                a_sc()
            if n >= 16 and n % 4 == 1 and nex < 16:
                a_ex[nex](gate_fn)
                nex += 1
            if n in (26, 47, 61):
                gi = {26: 0, 47: 2, 61: 4}[n]
                b_scores(GROUPS[gi])
                b_scores(GROUPS[gi + 1])
            if n in (33, 54, 68):
                b_softmax(GROUPS[{33: 0, 54: 2, 68: 4}[n]])
            if n in (38, 59, 73):
                b_softmax(GROUPS[{38: 1, 59: 3, 73: 5}[n]])
            if n == 84:
                a_pv()
            while pend and ready_after[pend[0]] <= n:
                b_pv(pend.pop(0))
        ex = extra_tasks(j, i)
        k = 0
        for g in pend:
            for _ in range(6):
                ex(k)()
                k += 1
            b_pv(g)
        for _ in range(8):
            ex(k)()
            k += 1
        fin()
        while k < NQUART:
            ex(k)()
            k += 1
        for t in post:
            t()

    def mix_tasks(jb, slot):
        def mix():
            ot = obuf[slot].reshape(512, BLK)
            a = _dot(woat[...], ot)
            b = bbuf[slot].T[:D].astype(F32)
            g = gsig[jb][0:1]
            outb[slot] = (g * a + (1.0 - g) * b).astype(BF16)

        def out():
            dst = out_h.at[:, pl.ds(pl.multiple_of(jb * BLK, BLK), BLK)]
            cp(outb.at[slot], dst, osem).wait()
            cp(outb.at[slot], dst, osem).start()
        return mix, out

    bbuf[1] = jnp.zeros((BLK, 512), BF16)
    obuf[1] = jnp.zeros((4, 128, BLK), BF16)
    outb[0] = jnp.zeros((D, BLK), BF16)
    cp(outb.at[0], out_h.at[:, pl.ds(0, BLK)], osem).start()

    def block(j, carry):
        jp = jnp.maximum(j - 1, 0)
        mix, out = mix_tasks(jp, (j + 1) % 2)
        jn = jnp.minimum(j + 1, NBLK - 1)
        for i in range(4):
            a_sc, a_ex, a_pv = a_attn_tasks(jn, (j + 1) % 2, i, j % 2, 1 - (j + 1) % 2)
            pre = [mix] if i == 0 else []
            post = [out] if i == 3 else []
            segment(j, i, (a_sc, a_ex, a_pv, pre, post))
        return carry

    jax.lax.fori_loop(0, NBLK, block, 0)

    mix, out = mix_tasks(NBLK - 1, (NBLK - 1) % 2)
    mix()
    out()
    cp(outb.at[0], out_h.at[:, pl.ds(0, BLK)], osem).wait()


@functools.partial(jax.jit, static_argnames=("B_seg_len",))
def pallas_gated_mix__sliding_block__memory_aug_recurrent_mem_tr__prompt_kernel(A_x, A_wqkv, A_wo, B_x, B_mem0, B_Wq, B_Wk, B_Wv, B_Wo, B_seg_len, gate_w):
    assert B_seg_len == SEG
    hbm = pl.BlockSpec(memory_space=pltpu.HBM)
    scratch = [
        pltpu.VMEM((D, S), BF16),
        pltpu.VMEM((D, 3 * D), BF16),
        pltpu.VMEM((D, D), BF16),
        pltpu.VMEM((D,), BF16),
        pltpu.VMEM((S + 8, D), BF16),
        pltpu.VMEM((MEM, D), BF16),
        pltpu.VMEM((3, 2, NRC, H * RC, 128), BF16),
        pltpu.VMEM((H * D, DHB), BF16),
        pltpu.VMEM((NTILES, D // 2, 128), U32),
        pltpu.VMEM((NHT, D // 2, 128), U32),
        pltpu.VMEM((NHT, D // 2, 128), U32),
        pltpu.VMEM((NHT, D // 2, 128), U32),
        pltpu.VMEM((D, 128), F32),
        pltpu.VMEM((4, D, 128), BF16),
        pltpu.VMEM((512, D), U32),
        pltpu.VMEM((D, 512), BF16),
        pltpu.VMEM((4, S + WIN, 128), BF16),
        pltpu.VMEM((NBLK, 4, 128, 128), BF16),
        pltpu.VMEM((NBLK + 2, 4, 128, 128), BF16),
        pltpu.VMEM((NBLK, 8, 128), F32),
        pltpu.VMEM((2, 4, 128, 128), BF16),
        pltpu.VMEM((2, 4, 3 * BLK, 128), F32),
        pltpu.VMEM((4, 3 * BLK, 128), BF16),
        pltpu.VMEM((NTILES, 2, 4 * L, 128), BF16),
        pltpu.VMEM((2, 6, 48, 128), BF16),
        pltpu.VMEM((2, BLK, 512), BF16),
        pltpu.VMEM((2, D, BLK), BF16),
        pltpu.SMEM((1,), jnp.int32),
        pltpu.SemaphoreType.DMA((9,)),
        pltpu.SemaphoreType.DMA(()),
    ]
    out_t = pl.pallas_call(
        _kernel,
        out_shape=jax.ShapeDtypeStruct((D, S), BF16),
        in_specs=[hbm] * 9,
        out_specs=hbm,
        scratch_shapes=scratch,
        compiler_params=pltpu.CompilerParams(vmem_limit_bytes=100 * 1024 * 1024),
    )(
        A_x.reshape(S, D).T, A_wqkv, A_wo, B_mem0.reshape(MEM, D),
        B_Wq.reshape(D * H, DHB), B_Wk.reshape(D * H, DHB), B_Wv.reshape(D * H, DHB),
        jnp.transpose(B_Wo, (0, 2, 1)).reshape(H * D, DHB), gate_w,
    )
    return out_t.T.reshape(1, S, D)
```

```python
import functools

import jax
import jax.numpy as jnp
import jax.experimental.pallas as pl
import jax.experimental.pallas.tpu as pltpu

F32 = jnp.float32
BF16 = jnp.bfloat16
U32 = jnp.uint32

NT = (((1,), (1,)), ((), ()))

S = 2048
D = 448
H = 16
DHA = 28
DHB = 256
MEM = 8
SEG = 32
L = MEM + SEG
BLK = 128
NBLK = S // BLK
WIN = 256
NHT = H * DHB // 128
NFT = H * D // 128
NTILES = 2 * NFT
NQUART = NTILES // 4
RC = 112
NRC = D // RC
NEG = -1e9
SCALE_A = 0.189453125
SCALE_B = 0.0625
GROUPS = [(0, 2, 4), (1, 3, 5), (6, 8, 10), (7, 9, 11), (12, 14), (13, 15)]


def _dot(a, b):
    return jnp.dot(a, b, preferred_element_type=F32)


def _dotg(a, b, dims):
    return jax.lax.dot_general(a, b, dims, preferred_element_type=F32)


def _kernel(xat_h, wqkv_h, woa_h, mem0_h, wq_h, wk_h, wv_h, wot_h, gate_h,
            out_h,
            xat, wqkv, woa, gate, xb, mem, raw, wot, wbig, wsq, wsk, wsv, shared,
            wka, wqvt, woat, ka, qt, vt, gsig, obuf, sbuf, mxb, pbuf, xp, ptb, bbuf, outb,
            zsm, sems, osem):
    cp = pltpu.make_async_copy
    zsm[0] = 0

    def zero_like_bits(v):
        return pltpu.bitcast(v, U32) & zsm[0].astype(U32)

    c_wqkv = cp(wqkv_h, wqkv, sems.at[0])
    c_xa = cp(xat_h, xat, sems.at[1])
    c_woa = cp(woa_h, woa, sems.at[2])
    c_gate = cp(gate_h, gate, sems.at[3])
    c_mem = cp(mem0_h, mem, sems.at[4])
    c_wo = cp(wot_h, wot, sems.at[5])

    def c_w(m, src):
        return [cp(src.at[pl.ds(H * RC * r, H * RC), pl.ds(128 * c, 128)], raw.at[m, c, r], sems.at[6 + m])
                for c in range(2) for r in range(NRC)]

    c_wv, c_wq, c_wk = c_w(0, wv_h), c_w(1, wq_h), c_w(2, wk_h)
    c_wqkv.start()
    c_wqkv.wait()
    for c in [c_xa, c_gate, c_woa, c_mem]:
        c.start()

    nrow = jax.lax.broadcasted_iota(jnp.int32, (1, 128), 1)
    trow = jnp.where(nrow % 32 < DHA, DHA * (nrow // 32) + nrow % 32, -4096)
    ncol = jax.lax.broadcasted_iota(jnp.int32, (128, 1), 0)
    tcol = jnp.where(ncol % 32 < DHA, DHA * (ncol // 32) + ncol % 32, -4096)
    for p in (0, 2, 1):
        for g in range(4):
            col0 = p * D + 112 * g
            start = (col0 // 128) * 128
            width = min(256, 3 * D - start)
            win = wqkv[:, pl.ds(start, width)]
            if p == 1:
                ci = jax.lax.broadcasted_iota(jnp.int32, (width, 128), 0)
                sel = jnp.where(ci == trow + (col0 - start), 1.0, 0.0).astype(BF16)
                wka[g] = _dot(win, sel).astype(BF16)
            else:
                cit = jax.lax.broadcasted_iota(jnp.int32, (128, width), 1)
                selt = jnp.where(cit == tcol + (col0 - start), 1.0, 0.0).astype(BF16)
                row0 = (0 if p == 0 else 512) + 128 * g
                wqvt[pl.ds(row0 // 2, 64), :] = pltpu.bitcast(_dotg(selt, win, NT).astype(BF16), U32)

    lane = jax.lax.broadcasted_iota(jnp.int32, (WIN, 128), 1)
    zk = jnp.where(lane % 32 == DHA, NEG, 0.0).astype(BF16)
    for g in range(4):
        ka[g, pl.ds(0, WIN), :] = zk
    for kb in range(2):
        vt[kb] = jnp.zeros((4, 128, 128), BF16)
    c_gate.wait()
    c_woa.wait()
    cj = jax.lax.broadcasted_iota(jnp.int32, (128, 112), 1)
    selo = jnp.where(cj == tcol, 1.0, 0.0).astype(BF16)
    for g in range(4):
        wop = _dot(selo, woa[pl.ds(112 * g, 112), :]).astype(BF16)
        woat[:, pl.ds(128 * g, 128)] = wop.T

    def gated(lhs, zbits):
        if zbits is None:
            return lhs
        head = pltpu.bitcast(pltpu.bitcast(lhs[0:16, 0:128], U32) | zbits, BF16)
        top = jnp.concatenate([head, lhs[0:16, 128:]], axis=1)
        return jnp.concatenate([top, lhs[16:]], axis=0)

    def a_proj_tasks(jb):
        r0 = pl.multiple_of(jb * BLK, BLK)
        st = {}

        def tr():
            xb[pl.ds(r0, BLK), :] = xat[:, pl.ds(r0, BLK)].T

        def qv(k):
            def f(zbits):
                lhs = gated(pltpu.bitcast(wqvt[pl.ds(128 * k, 128), :], BF16), zbits)
                y = _dot(lhs, xat[:, pl.ds(r0, BLK)])
                st['last'] = y[0:1]
                st['probe'] = [y[64 * c:64 * c + 1] for c in range(4)]
                for gg in range(2):
                    g = (2 * k + gg) % 4
                    yg = y[128 * gg:128 * (gg + 1)]
                    if k < 2:
                        qpad = jax.lax.broadcasted_iota(jnp.int32, (128, BLK), 0) % 32 == DHA
                        qt[jb, g] = jnp.where(qpad, 1.0, yg * SCALE_A).astype(BF16)
                    else:
                        vt[jb + 2, g] = yg.astype(BF16)
            return f

        def kk(k):
            def f(zbits):
                if k == 0:
                    gate8 = jnp.broadcast_to(gate[...].reshape(1, D), (8, D))
                    gsig[jb] = jax.nn.sigmoid(_dot(gate8, xat[:, pl.ds(r0, BLK)]))
                xblk = gated(xb[pl.ds(r0, BLK), :], zbits)
                for g in (2 * k, 2 * k + 1):
                    y = _dot(xblk, wka[g])
                    st['last'] = y[0:1]
                    st['probe'] = [y[32 * c:32 * c + 1] for c in range(4)]
                    ka[g, pl.ds(WIN + r0, BLK), :] = y.astype(BF16)
            return f

        def gate_fn(c=None):
            v = st['last'] if c is None else st['probe'][c]
            return pltpu.bitcast(zero_like_bits(v), F32)

        return tr, [qv(0), qv(1), qv(2), qv(3), kk(0), kk(1)], gate_fn

    def a_scores_tasks(jb, g, sa, kbs=(0, 1, 2)):
        st = {}

        def part(x, kb):
            def f():
                kr = jax.lax.broadcasted_iota(jnp.int32, (BLK, BLK), 0)
                qc = jax.lax.broadcasted_iota(jnp.int32, (BLK, BLK), 1)
                kblk = ka[g, pl.ds(pl.multiple_of((jb + kb) * BLK, BLK), BLK), :]
                for hh in range(4):
                    qs = qt[jb, g, pl.ds(32 * hh, 32), :]
                    parts = []
                    if hh > 0:
                        parts.append(jnp.zeros((32 * hh, BLK), BF16))
                    parts.append(qs)
                    if hh < 3:
                        parts.append(jnp.zeros((96 - 32 * hh, BLK), BF16))
                    sk = _dot(kblk, jnp.concatenate(parts, axis=0))
                    if kb == 0:
                        sk = jnp.where(kr > qc, sk, NEG)
                    elif kb == 2:
                        sk = jnp.where(kr <= qc, sk, NEG)
                    sbuf[sa, hh, pl.ds(BLK * x, BLK), :] = sk
                    mx = jnp.max(sk, axis=0, keepdims=True)
                    st[hh] = mx if x == 0 else jnp.maximum(st[hh], mx)
                    if x == len(kbs) - 1:
                        mxb[sa, hh] = jnp.broadcast_to(st[hh], (8, BLK))
            return f
        return [part(x, kb) for x, kb in enumerate(kbs)]

    def a_rest_tasks(jb, slot, g, sb, kbs=(0, 1, 2)):
        nk = BLK * len(kbs)
        ch = nk // 4
        st = {}

        def expo(hh, c):
            def f(gate_fn):
                mx = mxb[sb, hh][0:1] + gate_fn()
                e = jnp.exp(sbuf[sb, hh, pl.ds(ch * c, ch), :] - mx)
                part = jnp.sum(e, axis=0, keepdims=True)
                st[('l', hh)] = part if c == 0 else st[('l', hh)] + part
                pbuf[hh, pl.ds(ch * c, ch), :] = e.astype(BF16)
            return f

        def pv():
            for hh in range(4):
                vwin = jnp.concatenate(
                    [vt[jb + kb, g, pl.ds(32 * hh, 32), :] for kb in kbs], axis=1)
                o = _dot(vwin, pbuf[hh, pl.ds(0, nk), :]) / st[('l', hh)]
                obuf[slot, g, pl.ds(32 * hh, 32), :] = o.astype(BF16)

        return [expo(hh, c) for hh in range(4) for c in range(4)], pv

    raw32 = raw.bitcast(U32)

    def get_w(n):
        return pltpu.bitcast(wbig[n], BF16)

    def put_w(n, val):
        wbig[n] = pltpu.bitcast(val.astype(BF16), U32)

    def relay_chunk(m, dst, r, j, c, zf=None):
        a = raw32[m, c, r, pl.ds(j, RC, stride=8), :]
        if zf is not None:
            a = a | zf
        lo = pltpu.bitcast(a << 16, F32).astype(BF16)
        hi = pltpu.bitcast(a & jnp.uint32(0xFFFF0000), F32).astype(BF16)
        lo, hi = pltpu.bitcast(lo, U32), pltpu.bitcast(hi, U32)
        rows = pl.ds(pl.multiple_of(RC // 2 * r, 8), RC // 2)
        dst[4 * j + c, rows, :] = lo
        dst[4 * j + 2 + c, rows, :] = hi
        return lo[RC // 2 - 8:] | hi[RC // 2 - 8:]

    def a_proj_loop(lo, hi, m, with_attn, pre=None):
        def body(jb, carry):
            if pre is not None:
                pre(jb)
            tr, stages, gate_fn = a_proj_tasks(jb)
            jc = [(j, c) for j in range(8) for c in range(2)]
            split = [0, 4, 8, 12, 16, 16, 16]
            asplit = [0, 3, 6, 9, 12, 16, 16]
            if with_attn:
                a_ex, a_pv = a_rest_tasks(0, 0, jb % 4, (jb + 16) // 32, kbs=(2,))
            tr()
            if with_attn:
                for t in a_scores_tasks(0, jb % 4, jb // 16, kbs=(2,)):
                    t()
            due = [None] * 8
            for k, stage in enumerate(stages):
                zin = due[k]
                if k > 0:
                    chain = pltpu.bitcast(gate_fn(), U32)
                    chain = jnp.broadcast_to(chain, (8, 128))
                    zin = chain if zin is None else zin | chain
                stage(zin)
                z = None
                if m is not None:
                    mm, base = m(jb)
                    for ci, (j, c) in enumerate(jc[split[k]:split[k + 1]]):
                        zz = relay_chunk(mm, base, jb % NRC, j, c, pltpu.bitcast(gate_fn(ci % 4), U32))
                        z = zz if z is None else z | zz
                    if z is not None:
                        due[min(k + 2, 5)] = (z & zsm[0].astype(U32)) if due[min(k + 2, 5)] is None else (z & zsm[0].astype(U32)) | due[min(k + 2, 5)]
                if with_attn and k < 5:
                    for t in a_ex[asplit[k]:asplit[k + 1]]:
                        t(gate_fn)
            if with_attn:
                a_pv()
            return carry
        jax.lax.fori_loop(lo, hi, body, 0)

    def starter(at, copies):
        def pre(jb):
            @pl.when(jb == at)
            def _():
                for c in copies:
                    c.start()
        return pre

    c_xa.wait()
    for c in c_wv:
        c.start()
    a_proj_loop(0, 8, None, False, starter(4, c_wq))
    c_wo.start()
    for c in c_wv:
        c.wait()
    a_proj_loop(8, 12, lambda jb: (0, wsv), True, starter(10, c_wk))
    for c in c_wq:
        c.wait()
    a_proj_loop(12, 16, lambda jb: (1, wsq), False)

    def xrow(r):
        return (r // SEG) * L + MEM + r % SEG

    XR0 = (0, 40, 64, 104, 128)

    def main_tasks(j, i):
        nx = XR0[i + 1] - XR0[i]
        src = pl.multiple_of(j * BLK + XR0[i], 8)
        st = {}

        def prep():
            st['lhs'] = jnp.concatenate([mem[...], xb[pl.ds(src, nx), :]], axis=0)

        def tile(n):
            y32 = _dot(st['lhs'], get_w(n))
            st['last'] = y32[0:1]
            y = y32.astype(BF16)
            xp[n, pl.ds(L * i, 8), :] = y[0:8]
            for t in range(nx // 8):
                xp[n, pl.ds(xrow(XR0[i] + 8 * t), 8), :] = y[8 + 8 * t:16 + 8 * t]

        def gate_fn():
            return pltpu.bitcast(zero_like_bits(st['last']), F32)
        return prep, tile, gate_fn, (lambda: st['lhs'][0:MEM])

    c_mem.wait()
    c_wo.wait()
    z64 = jnp.zeros((64, DHB), BF16)

    def head_w(src, h):
        return jnp.concatenate([pltpu.bitcast(src[2 * h], BF16), pltpu.bitcast(src[2 * h + 1], BF16)], axis=1)

    def fold_mm(kind, j, odd, half):
        h = 2 * j + odd
        if kind == 0:
            t0, lhs, w = 7 * j, head_w(wsq, h), head_w(wsk, h)
        else:
            t0, lhs, w = NFT + 7 * j, head_w(wsv, h), wot[pl.ds(pl.multiple_of(D * h, 64), D), :]
        w = jnp.concatenate([z64, w] if odd else [w, z64], axis=0)[256 * half:256 * half + 256]
        b = _dotg(lhs, w, NT)
        if kind == 0:
            b = b * SCALE_B
        if not odd:
            put_w(t0 + 2 * half, b[:, 0:128])
            if half == 0:
                put_w(t0 + 1, b[:, 128:256])
            else:
                shared[...] = b[:, 128:256]
        else:
            if half == 0:
                put_w(t0 + 3, shared[...] + b[:, 0:128])
            else:
                put_w(t0 + 5, b[:, 0:128])
            put_w(t0 + 4 + 2 * half, b[:, 128:256])
        return [zero_like_bits(b[112 * c:112 * c + 1, 0:128]) for c in range(4)]

    for c in c_wk:
        c.wait()

    def u_fold(r, carry):
        kch = [(jj, c) for jj in range(8) for c in range(2)]
        nk = 0
        for jp in range(2):
            for odd in range(2):
                for half in range(2):
                    probes = fold_mm(1, 2 * r + jp, odd, half)
                    for pz in probes[1:3]:
                        relay_chunk(2, wsk, r, kch[nk][0], kch[nk][1], pz)
                        nk += 1
        return carry

    jax.lax.fori_loop(0, NRC, u_fold, 0)

    def t_fold(j, carry):
        for odd in range(2):
            for half in range(2):
                fold_mm(0, j, odd, half)
        return carry

    jax.lax.fori_loop(0, 8, t_fold, 0, unroll=2)

    def segment(j, i, atasks):
        st = {'acc': [None, None]}
        ptslot_w = j % 2
        ptslot_r = 1 - (j + 1) % 2
        prep, mtile, gate_fn, mem0_val = main_tasks(j, i)

        def xt(n):
            return xp[n, pl.ds(L * i, L), :]

        def window(base, h):
            return jnp.concatenate([xt(base + (7 * h) // 2 + t) for t in range(4)], axis=1)

        def b_scores(grp):
            if 'hp' not in st:
                r = pl.multiple_of((4 * j + i) * SEG, SEG)
                hrows = jnp.concatenate([mem0_val(), xb[pl.ds(r, SEG), :]], axis=0)
                z = jnp.zeros((L, 64), BF16)
                st['hp'] = [jnp.concatenate([hrows, z], axis=1), jnp.concatenate([z, hrows], axis=1)]
            t = jnp.concatenate([window(0, h) for h in grp], axis=0)
            st[grp] = _dotg(st['hp'][grp[0] % 2], t, NT)

        def b_softmax(grp):
            n = len(grp)
            row = jax.lax.broadcasted_iota(jnp.int32, (L, L * n), 0)
            lane = jax.lax.broadcasted_iota(jnp.int32, (L, L * n), 1)
            blk = [(lane >= L * a) & (lane < L * (a + 1)) for a in range(n)]
            t = lane
            for a in range(1, n):
                t = jnp.where(lane >= L * a, lane - L * a, t)
            s = jnp.where((t < MEM) | (t >= row), st[grp], NEG)
            mx = jnp.max(s, axis=0, keepdims=True)
            e = jnp.exp(s - mx)
            l = jnp.sum(e, axis=0, keepdims=True)
            p = e * (1.0 / l)
            blocks = [jnp.where(blk[a], p, 0.0) for a in range(n)]
            blocks.append(jnp.zeros((128 - L * n, L * n), F32))
            p = jnp.concatenate(blocks, axis=0)
            p = jnp.concatenate([p, jnp.zeros((128, 128 - L * n), F32)], axis=1).T
            lhs = p[0:L]
            for a in range(1, n):
                lhs = lhs + p[L * a:L * (a + 1)]
            lhs = jnp.concatenate([lhs, jnp.zeros((8, 128), F32)], axis=0)
            ptb[ptslot_w, GROUPS.index(grp)] = lhs.astype(BF16)

        def b_pv(grp):
            par = grp[0] % 2
            kk = L * len(grp)
            p = ptb[ptslot_r, GROUPS.index(grp)][:L, :kk]
            u = jnp.concatenate([window(NFT, h) for h in grp], axis=0)
            o = _dot(p, u)
            st['acc'][par] = o if st['acc'][par] is None else st['acc'][par] + o

        def fin():
            a0, a1 = st['acc']
            o = a0 + jnp.concatenate([a1[:, 64:512], jnp.zeros((L, 64), F32)], axis=1)
            ob = o.astype(BF16)
            mem[...] = ob[0:MEM, :D]
            bbuf[j % 2, pl.ds(SEG * i, SEG), :] = ob[MEM:]

        a_ex, a_pv, a_next, mid, post = atasks
        lag = 6 if i % 2 else 4
        prep()
        nex = 0
        ready_after = {g: NFT + (7 * max(g)) // 2 + 3 + lag for g in GROUPS}
        pend = list(GROUPS)
        for n in range(NTILES):
            mtile(n)
            if n >= 4 and n % 4 == 1 and nex < 16:
                a_ex[nex](gate_fn)
                nex += 1
            if n in (26, 47, 61):
                gi = {26: 0, 47: 2, 61: 4}[n]
                b_scores(GROUPS[gi])
                b_scores(GROUPS[gi + 1])
            if n in (33, 54, 68):
                b_softmax(GROUPS[{33: 0, 54: 2, 68: 4}[n]])
            if n in (38, 59, 73):
                b_softmax(GROUPS[{38: 1, 59: 3, 73: 5}[n]])
            if n == 76:
                a_pv()
            while pend and ready_after[pend[0]] <= n:
                b_pv(pend.pop(0))
        a_next[0]()
        for g in pend:
            b_pv(g)
        a_next[1]()
        for t in mid:
            t()
        a_next[2]()
        fin()
        for t in post:
            t()

    def mix_tasks(jb, slot, oslot):
        def mix():
            ot = obuf[oslot].reshape(512, BLK)
            a = _dot(woat[...], ot)
            b = bbuf[slot].T[:D].astype(F32)
            g = gsig[jb][0:1]
            outb[slot] = (g * a + (1.0 - g) * b).astype(BF16)

        def out():
            dst = out_h.at[:, pl.ds(pl.multiple_of(jb * BLK, BLK), BLK)]
            cp(outb.at[slot], dst, osem).wait()
            cp(outb.at[slot], dst, osem).start()
        return mix, out

    bbuf[1] = jnp.zeros((BLK, 512), BF16)
    obuf[2] = jnp.zeros((4, 128, BLK), BF16)
    outb[0] = jnp.zeros((D, BLK), BF16)
    cp(outb.at[0], out_h.at[:, pl.ds(0, BLK)], osem).start()

    for t in a_scores_tasks(1, 0, 0):
        t()

    def block(j, carry):
        jp = jnp.maximum(j - 1, 0)
        mix, out = mix_tasks(jp, (j + 1) % 2, (j + 2) % 3)
        jn = jnp.minimum(j + 1, NBLK - 1)
        jn2 = jnp.minimum(j + 2, NBLK - 1)
        zero = j // NBLK
        for i in range(4):
            a_ex, a_pv = a_rest_tasks(jn, (j + 1) % 3, i, i % 2 + zero)
            if i < 3:
                a_next = a_scores_tasks(jn, i + 1, (i + 1) % 2)
            else:
                a_next = a_scores_tasks(jn2, 0, 0)
            mid = [mix] if i == 0 else []
            post = [out] if i == 3 else []
            segment(j, i, (a_ex, a_pv, a_next, mid, post))
        return carry

    jax.lax.fori_loop(0, NBLK, block, 0)

    mix, out = mix_tasks(NBLK - 1, (NBLK - 1) % 2, (NBLK - 1) % 3)
    mix()
    out()
    cp(outb.at[0], out_h.at[:, pl.ds(0, BLK)], osem).wait()


@functools.partial(jax.jit, static_argnames=("B_seg_len",))
def pallas_gated_mix__sliding_block__memory_aug_recurrent_mem_tr__prompt_kernel(A_x, A_wqkv, A_wo, B_x, B_mem0, B_Wq, B_Wk, B_Wv, B_Wo, B_seg_len, gate_w):
    assert B_seg_len == SEG
    hbm = pl.BlockSpec(memory_space=pltpu.HBM)
    scratch = [
        pltpu.VMEM((D, S), BF16),
        pltpu.VMEM((D, 3 * D), BF16),
        pltpu.VMEM((D, D), BF16),
        pltpu.VMEM((D,), BF16),
        pltpu.VMEM((S + 8, D), BF16),
        pltpu.VMEM((MEM, D), BF16),
        pltpu.VMEM((3, 2, NRC, H * RC, 128), BF16),
        pltpu.VMEM((H * D, DHB), BF16),
        pltpu.VMEM((NTILES, D // 2, 128), U32),
        pltpu.VMEM((NHT, D // 2, 128), U32),
        pltpu.VMEM((NHT, D // 2, 128), U32),
        pltpu.VMEM((NHT, D // 2, 128), U32),
        pltpu.VMEM((D, 128), F32),
        pltpu.VMEM((4, D, 128), BF16),
        pltpu.VMEM((512, D), U32),
        pltpu.VMEM((D, 512), BF16),
        pltpu.VMEM((4, S + WIN, 128), BF16),
        pltpu.VMEM((NBLK, 4, 128, 128), BF16),
        pltpu.VMEM((NBLK + 2, 4, 128, 128), BF16),
        pltpu.VMEM((NBLK, 8, 128), F32),
        pltpu.VMEM((3, 4, 128, 128), BF16),
        pltpu.VMEM((2, 4, 3 * BLK, 128), F32),
        pltpu.VMEM((2, 4, 8, BLK), F32),
        pltpu.VMEM((4, 3 * BLK, 128), BF16),
        pltpu.VMEM((NTILES, 4 * L, 128), BF16),
        pltpu.VMEM((2, 6, 48, 128), BF16),
        pltpu.VMEM((2, BLK, 512), BF16),
        pltpu.VMEM((2, D, BLK), BF16),
        pltpu.SMEM((1,), jnp.int32),
        pltpu.SemaphoreType.DMA((9,)),
        pltpu.SemaphoreType.DMA(()),
    ]
    out_t = pl.pallas_call(
        _kernel,
        out_shape=jax.ShapeDtypeStruct((D, S), BF16),
        in_specs=[hbm] * 9,
        out_specs=hbm,
        scratch_shapes=scratch,
        compiler_params=pltpu.CompilerParams(vmem_limit_bytes=100 * 1024 * 1024),
    )(
        A_x.reshape(S, D).T, A_wqkv, A_wo, B_mem0.reshape(MEM, D),
        B_Wq.reshape(D * H, DHB), B_Wk.reshape(D * H, DHB), B_Wv.reshape(D * H, DHB),
        jnp.transpose(B_Wo, (0, 2, 1)).reshape(H * D, DHB), gate_w,
    )
    return out_t.T.reshape(1, S, D)
```

```python
import functools

import jax
import jax.numpy as jnp
import jax.experimental.pallas as pl
import jax.experimental.pallas.tpu as pltpu

F32 = jnp.float32
BF16 = jnp.bfloat16
U32 = jnp.uint32

NT = (((1,), (1,)), ((), ()))

S = 2048
D = 448
H = 16
DHA = 28
DHB = 256
MEM = 8
SEG = 32
L = MEM + SEG
BLK = 128
NBLK = S // BLK
WIN = 256
NHT = H * DHB // 128
NFT = H * D // 128
NTILES = 2 * NFT
NQUART = NTILES // 4
RC = 112
NRC = D // RC
NEG = -1e9
SCALE_A = 0.189453125
SCALE_B = 0.0625
GROUPS = [(0, 2, 4), (1, 3, 5), (6, 8, 10), (7, 9, 11), (12, 14), (13, 15)]


def _dot(a, b):
    return jnp.dot(a, b, preferred_element_type=F32)


def _dotg(a, b, dims):
    return jax.lax.dot_general(a, b, dims, preferred_element_type=F32)


def _kernel(xat_h, wqkv_h, woa_h, mem0_h, wq_h, wk_h, wv_h, wot_h, gate_h,
            out_h,
            xat, wqkv, woa, gate, xb, mem, raw, wot, wbig, wsq, wsk, wsv, shared,
            wka, wqvt, woat, ka, qt, vt, gsig, obuf, sbuf, mxb, pbuf, xp, ptb, bbuf, outb,
            zsm, sems, osem):
    cp = pltpu.make_async_copy
    zsm[0] = 0

    def zero_like_bits(v):
        return pltpu.bitcast(v, U32) & zsm[0].astype(U32)

    c_wqkv = cp(wqkv_h, wqkv, sems.at[0])
    c_xa = cp(xat_h, xat, sems.at[1])
    c_woa = cp(woa_h, woa, sems.at[2])
    c_gate = cp(gate_h, gate, sems.at[3])
    c_mem = cp(mem0_h, mem, sems.at[4])
    c_wo = cp(wot_h, wot, sems.at[5])

    def c_w(m, src):
        return [cp(src.at[pl.ds(H * RC * r, H * RC), pl.ds(128 * c, 128)], raw.at[m, c, r], sems.at[6 + m])
                for c in range(2) for r in range(NRC)]

    c_wv, c_wq, c_wk = c_w(0, wv_h), c_w(1, wq_h), c_w(2, wk_h)
    c_wqkv.start()
    c_wqkv.wait()
    for c in [c_xa, c_gate, c_woa, c_mem]:
        c.start()

    nrow = jax.lax.broadcasted_iota(jnp.int32, (1, 128), 1)
    trow = jnp.where(nrow % 32 < DHA, DHA * (nrow // 32) + nrow % 32, -4096)
    ncol = jax.lax.broadcasted_iota(jnp.int32, (128, 1), 0)
    tcol = jnp.where(ncol % 32 < DHA, DHA * (ncol // 32) + ncol % 32, -4096)
    for p in (0, 2, 1):
        for g in range(4):
            col0 = p * D + 112 * g
            start = (col0 // 128) * 128
            width = min(256, 3 * D - start)
            win = wqkv[:, pl.ds(start, width)]
            if p == 1:
                ci = jax.lax.broadcasted_iota(jnp.int32, (width, 128), 0)
                sel = jnp.where(ci == trow + (col0 - start), 1.0, 0.0).astype(BF16)
                wka[g] = _dot(win, sel).astype(BF16)
            else:
                cit = jax.lax.broadcasted_iota(jnp.int32, (128, width), 1)
                selt = jnp.where(cit == tcol + (col0 - start), 1.0, 0.0).astype(BF16)
                row0 = (0 if p == 0 else 512) + 128 * g
                wqvt[pl.ds(row0 // 2, 64), :] = pltpu.bitcast(_dotg(selt, win, NT).astype(BF16), U32)

    lane = jax.lax.broadcasted_iota(jnp.int32, (WIN, 128), 1)
    zk = jnp.where(lane % 32 == DHA, NEG, 0.0).astype(BF16)
    for g in range(4):
        ka[g, pl.ds(0, WIN), :] = zk
    for kb in range(2):
        vt[kb] = jnp.zeros((4, 128, 128), BF16)
    c_gate.wait()
    c_woa.wait()
    cj = jax.lax.broadcasted_iota(jnp.int32, (128, 112), 1)
    selo = jnp.where(cj == tcol, 1.0, 0.0).astype(BF16)
    for g in range(4):
        wop = _dot(selo, woa[pl.ds(112 * g, 112), :]).astype(BF16)
        woat[:, pl.ds(128 * g, 128)] = wop.T

    def gated(lhs, zbits):
        if zbits is None:
            return lhs
        head = pltpu.bitcast(pltpu.bitcast(lhs[0:16, 0:128], U32) | zbits, BF16)
        top = jnp.concatenate([head, lhs[0:16, 128:]], axis=1)
        return jnp.concatenate([top, lhs[16:]], axis=0)

    def a_proj_tasks(jb):
        r0 = pl.multiple_of(jb * BLK, BLK)
        st = {}

        def tr():
            xb[pl.ds(r0, BLK), :] = xat[:, pl.ds(r0, BLK)].T

        def qv(k):
            def f(zbits):
                lhs = gated(pltpu.bitcast(wqvt[pl.ds(128 * k, 128), :], BF16), zbits)
                y = _dot(lhs, xat[:, pl.ds(r0, BLK)])
                st['last'] = y[0:1]
                st['probe'] = [y[64 * c:64 * c + 1] for c in range(4)]
                for gg in range(2):
                    g = (2 * k + gg) % 4
                    yg = y[128 * gg:128 * (gg + 1)]
                    if k < 2:
                        qpad = jax.lax.broadcasted_iota(jnp.int32, (128, BLK), 0) % 32 == DHA
                        qt[jb, g] = jnp.where(qpad, 1.0, yg * SCALE_A).astype(BF16)
                    else:
                        vt[jb + 2, g] = yg.astype(BF16)
            return f

        def kk(k):
            def f(zbits):
                if k == 0:
                    gate8 = jnp.broadcast_to(gate[...].reshape(1, D), (8, D))
                    gsig[jb] = jax.nn.sigmoid(_dot(gate8, xat[:, pl.ds(r0, BLK)]))
                xblk = gated(xb[pl.ds(r0, BLK), :], zbits)
                for g in (2 * k, 2 * k + 1):
                    y = _dot(xblk, wka[g])
                    st['last'] = y[0:1]
                    st['probe'] = [y[32 * c:32 * c + 1] for c in range(4)]
                    ka[g, pl.ds(WIN + r0, BLK), :] = y.astype(BF16)
            return f

        def gate_fn(c=None):
            v = st['last'] if c is None else st['probe'][c]
            return pltpu.bitcast(zero_like_bits(v), F32)

        return tr, [qv(0), qv(1), qv(2), qv(3), kk(0), kk(1)], gate_fn

    def a_scores_tasks(jb, g, sa, kbs=(0, 1, 2)):
        st = {}

        def part(x, kb):
            def f():
                kr = jax.lax.broadcasted_iota(jnp.int32, (BLK, BLK), 0)
                qc = jax.lax.broadcasted_iota(jnp.int32, (BLK, BLK), 1)
                kblk = ka[g, pl.ds(pl.multiple_of((jb + kb) * BLK, BLK), BLK), :]
                for hh in range(4):
                    qs = qt[jb, g, pl.ds(32 * hh, 32), :]
                    parts = []
                    if hh > 0:
                        parts.append(jnp.zeros((32 * hh, BLK), BF16))
                    parts.append(qs)
                    if hh < 3:
                        parts.append(jnp.zeros((96 - 32 * hh, BLK), BF16))
                    sk = _dot(kblk, jnp.concatenate(parts, axis=0))
                    if kb == 0:
                        sk = jnp.where(kr > qc, sk, NEG)
                    elif kb == 2:
                        sk = jnp.where(kr <= qc, sk, NEG)
                    sbuf[sa, hh, pl.ds(BLK * x, BLK), :] = sk
                    mx = jnp.max(sk, axis=0, keepdims=True)
                    st[hh] = mx if x == 0 else jnp.maximum(st[hh], mx)
                    if x == len(kbs) - 1:
                        mxb[sa, hh] = jnp.broadcast_to(st[hh], (8, BLK))
            return f
        return [part(x, kb) for x, kb in enumerate(kbs)]

    def a_rest_tasks(jb, slot, g, sb, kbs=(0, 1, 2)):
        nk = BLK * len(kbs)
        ch = nk // 4
        st = {}

        def expo(hh, c):
            def f(gate_fn):
                mx = mxb[sb, hh][0:1] + gate_fn()
                e = jnp.exp(sbuf[sb, hh, pl.ds(ch * c, ch), :] - mx)
                part = jnp.sum(e, axis=0, keepdims=True)
                st[('l', hh)] = part if c == 0 else st[('l', hh)] + part
                pbuf[hh, pl.ds(ch * c, ch), :] = e.astype(BF16)
            return f

        def pv():
            for hh in range(4):
                vwin = jnp.concatenate(
                    [vt[jb + kb, g, pl.ds(32 * hh, 32), :] for kb in kbs], axis=1)
                o = _dot(vwin, pbuf[hh, pl.ds(0, nk), :]) / st[('l', hh)]
                obuf[slot, g, pl.ds(32 * hh, 32), :] = o.astype(BF16)

        return [expo(hh, c) for hh in range(4) for c in range(4)], pv

    raw32 = raw.bitcast(U32)

    def get_w(n):
        return pltpu.bitcast(wbig[n], BF16)

    def put_w(n, val):
        wbig[n] = pltpu.bitcast(val.astype(BF16), U32)

    def relay_chunk(m, dst, r, j, c, zf=None):
        a = raw32[m, c, r, pl.ds(j, RC, stride=8), :]
        if zf is not None:
            a = a | zf
        lo = pltpu.bitcast(a << 16, F32).astype(BF16)
        hi = pltpu.bitcast(a & jnp.uint32(0xFFFF0000), F32).astype(BF16)
        lo, hi = pltpu.bitcast(lo, U32), pltpu.bitcast(hi, U32)
        rows = pl.ds(pl.multiple_of(RC // 2 * r, 8), RC // 2)
        dst[4 * j + c, rows, :] = lo
        dst[4 * j + 2 + c, rows, :] = hi
        return lo[RC // 2 - 8:] | hi[RC // 2 - 8:]

    def a_proj_loop(lo, hi, m, with_attn, pre=None, unroll=1):
        def body(jb, carry):
            if pre is not None:
                pre(jb)
            tr, stages, gate_fn = a_proj_tasks(jb)
            jc = [(j, c) for j in range(8) for c in range(2)]
            split = [0, 4, 8, 12, 16, 16, 16]
            asplit = [0, 3, 6, 9, 12, 16, 16]
            if with_attn:
                a_ex, a_pv = a_rest_tasks(0, 0, jb % 4, (jb + 16) // 32, kbs=(2,))
            tr()
            if with_attn:
                for t in a_scores_tasks(0, jb % 4, jb // 16, kbs=(2,)):
                    t()
            due = [None] * 8
            for k, stage in enumerate(stages):
                zin = due[k]
                if k > 0:
                    chain = pltpu.bitcast(gate_fn(), U32)
                    chain = jnp.broadcast_to(chain, (8, 128))
                    zin = chain if zin is None else zin | chain
                stage(zin)
                z = None
                if m is not None:
                    mm, base = m(jb)
                    for ci, (j, c) in enumerate(jc[split[k]:split[k + 1]]):
                        zz = relay_chunk(mm, base, jb % NRC, j, c, pltpu.bitcast(gate_fn(ci % 4), U32))
                        z = zz if z is None else z | zz
                    if z is not None:
                        due[min(k + 2, 5)] = (z & zsm[0].astype(U32)) if due[min(k + 2, 5)] is None else (z & zsm[0].astype(U32)) | due[min(k + 2, 5)]
                if with_attn and k < 5:
                    for t in a_ex[asplit[k]:asplit[k + 1]]:
                        t(gate_fn)
            if with_attn:
                a_pv()
            return carry
        jax.lax.fori_loop(lo, hi, body, 0, unroll=unroll)

    def starter(at, copies):
        def pre(jb):
            @pl.when(jb == at)
            def _():
                for c in copies:
                    c.start()
        return pre

    c_xa.wait()
    for c in c_wv:
        c.start()
    a_proj_loop(0, 8, None, False, starter(4, c_wq), unroll=1)
    c_wo.start()
    for c in c_wv:
        c.wait()
    a_proj_loop(8, 12, lambda jb: (0, wsv), True, starter(10, c_wk))
    for c in c_wq:
        c.wait()
    a_proj_loop(12, 16, lambda jb: (1, wsq), False, unroll=1)

    def xrow(r):
        return (r // SEG) * L + MEM + r % SEG

    XR0 = (0, 40, 64, 104, 128)

    def main_tasks(j, i):
        nx = XR0[i + 1] - XR0[i]
        src = pl.multiple_of(j * BLK + XR0[i], 8)
        st = {}

        def prep():
            st['lhs'] = jnp.concatenate([mem[...], xb[pl.ds(src, nx), :]], axis=0)

        def tile(n):
            y32 = _dot(st['lhs'], get_w(n))
            st['last'] = y32[0:1]
            y = y32.astype(BF16)
            xp[n, pl.ds(L * i, 8), :] = y[0:8]
            for t in range(nx // 8):
                xp[n, pl.ds(xrow(XR0[i] + 8 * t), 8), :] = y[8 + 8 * t:16 + 8 * t]

        def gate_fn():
            return pltpu.bitcast(zero_like_bits(st['last']), F32)
        return prep, tile, gate_fn, (lambda: st['lhs'][0:MEM])

    c_mem.wait()
    c_wo.wait()
    z64 = jnp.zeros((64, DHB), BF16)

    def head_w(src, h):
        return jnp.concatenate([pltpu.bitcast(src[2 * h], BF16), pltpu.bitcast(src[2 * h + 1], BF16)], axis=1)

    def fold_mm(kind, j, odd, half):
        h = 2 * j + odd
        if kind == 0:
            t0, lhs, w = 7 * j, head_w(wsq, h), head_w(wsk, h)
        else:
            t0, lhs, w = NFT + 7 * j, head_w(wsv, h), wot[pl.ds(pl.multiple_of(D * h, 64), D), :]
        w = jnp.concatenate([z64, w] if odd else [w, z64], axis=0)[256 * half:256 * half + 256]
        b = _dotg(lhs, w, NT)
        if kind == 0:
            b = b * SCALE_B
        if not odd:
            put_w(t0 + 2 * half, b[:, 0:128])
            if half == 0:
                put_w(t0 + 1, b[:, 128:256])
            else:
                shared[...] = b[:, 128:256]
        else:
            if half == 0:
                put_w(t0 + 3, shared[...] + b[:, 0:128])
            else:
                put_w(t0 + 5, b[:, 0:128])
            put_w(t0 + 4 + 2 * half, b[:, 128:256])
        return [zero_like_bits(b[112 * c:112 * c + 1, 0:128]) for c in range(4)]

    for c in c_wk:
        c.wait()

    def u_fold(r, carry):
        kch = [(jj, c) for jj in range(8) for c in range(2)]
        nk = 0
        for jp in range(2):
            for odd in range(2):
                for half in range(2):
                    probes = fold_mm(1, 2 * r + jp, odd, half)
                    for pz in probes[1:3]:
                        relay_chunk(2, wsk, r, kch[nk][0], kch[nk][1], pz)
                        nk += 1
        return carry

    jax.lax.fori_loop(0, NRC, u_fold, 0, unroll=1)

    def t_fold(j, carry):
        for odd in range(2):
            for half in range(2):
                fold_mm(0, j, odd, half)
        return carry

    jax.lax.fori_loop(0, 8, t_fold, 0, unroll=2)

    def segment(j, i, atasks):
        st = {'acc': [None, None]}
        ptslot_w = j % 2
        ptslot_r = 1 - (j + 1) % 2
        prep, mtile, gate_fn, mem0_val = main_tasks(j, i)

        def xt(n):
            return xp[n, pl.ds(L * i, L), :]

        def window(base, h):
            return jnp.concatenate([xt(base + (7 * h) // 2 + t) for t in range(4)], axis=1)

        def b_scores(grp):
            if 'hp' not in st:
                r = pl.multiple_of((4 * j + i) * SEG, SEG)
                hrows = jnp.concatenate([mem0_val(), xb[pl.ds(r, SEG), :]], axis=0)
                z = jnp.zeros((L, 64), BF16)
                st['hp'] = [jnp.concatenate([hrows, z], axis=1), jnp.concatenate([z, hrows], axis=1)]
            t = jnp.concatenate([window(0, h) for h in grp], axis=0)
            st[grp] = _dotg(st['hp'][grp[0] % 2], t, NT)

        def b_softmax(grp):
            n = len(grp)
            row = jax.lax.broadcasted_iota(jnp.int32, (L, L * n), 0)
            lane = jax.lax.broadcasted_iota(jnp.int32, (L, L * n), 1)
            blk = [(lane >= L * a) & (lane < L * (a + 1)) for a in range(n)]
            t = lane
            for a in range(1, n):
                t = jnp.where(lane >= L * a, lane - L * a, t)
            s = jnp.where((t < MEM) | (t >= row), st[grp], NEG)
            mx = jnp.max(s, axis=0, keepdims=True)
            e = jnp.exp(s - mx)
            l = jnp.sum(e, axis=0, keepdims=True)
            p = e * (1.0 / l)
            blocks = [jnp.where(blk[a], p, 0.0) for a in range(n)]
            blocks.append(jnp.zeros((128 - L * n, L * n), F32))
            p = jnp.concatenate(blocks, axis=0)
            p = jnp.concatenate([p, jnp.zeros((128, 128 - L * n), F32)], axis=1).T
            lhs = p[0:L]
            for a in range(1, n):
                lhs = lhs + p[L * a:L * (a + 1)]
            lhs = jnp.concatenate([lhs, jnp.zeros((8, 128), F32)], axis=0)
            ptb[ptslot_w, GROUPS.index(grp)] = lhs.astype(BF16)

        def b_pv(grp):
            par = grp[0] % 2
            kk = L * len(grp)
            p = ptb[ptslot_r, GROUPS.index(grp)][:L, :kk]
            u = jnp.concatenate([window(NFT, h) for h in grp], axis=0)
            o = _dot(p, u)
            st['acc'][par] = o if st['acc'][par] is None else st['acc'][par] + o

        def fin():
            a0, a1 = st['acc']
            o = a0 + jnp.concatenate([a1[:, 64:512], jnp.zeros((L, 64), F32)], axis=1)
            ob = o.astype(BF16)
            mem[...] = ob[0:MEM, :D]
            bbuf[j % 2, pl.ds(SEG * i, SEG), :] = ob[MEM:]

        a_ex, a_pv, a_next, mid, post = atasks
        lag = 8 if i % 2 else 6
        prep()
        nex = 0
        ready_after = {g: NFT + (7 * max(g)) // 2 + 3 + lag for g in GROUPS}
        pend = list(GROUPS)
        for n in range(NTILES):
            mtile(n)
            if n >= 4 and n % 4 == 1 and nex < 16:
                a_ex[nex](gate_fn)
                nex += 1
            if n in (26, 47, 61):
                gi = {26: 0, 47: 2, 61: 4}[n]
                b_scores(GROUPS[gi])
                b_scores(GROUPS[gi + 1])
            if n in (33, 54, 68):
                b_softmax(GROUPS[{33: 0, 54: 2, 68: 4}[n]])
            if n in (38, 59, 73):
                b_softmax(GROUPS[{38: 1, 59: 3, 73: 5}[n]])
            if n == 70:
                a_pv()
            while pend and ready_after[pend[0]] <= n:
                b_pv(pend.pop(0))
        a_next[0]()
        for g in pend:
            b_pv(g)
        a_next[1]()
        for t in mid:
            t()
        a_next[2]()
        fin()
        for t in post:
            t()

    def mix_tasks(jb, slot, oslot):
        def mix():
            ot = obuf[oslot].reshape(512, BLK)
            a = _dot(woat[...], ot)
            b = bbuf[slot].T[:D].astype(F32)
            g = gsig[jb][0:1]
            outb[slot] = (g * a + (1.0 - g) * b).astype(BF16)

        def out():
            dst = out_h.at[:, pl.ds(pl.multiple_of(jb * BLK, BLK), BLK)]
            cp(outb.at[slot], dst, osem).wait()
            cp(outb.at[slot], dst, osem).start()
        return mix, out

    bbuf[1] = jnp.zeros((BLK, 512), BF16)
    obuf[2] = jnp.zeros((4, 128, BLK), BF16)
    outb[0] = jnp.zeros((D, BLK), BF16)
    cp(outb.at[0], out_h.at[:, pl.ds(0, BLK)], osem).start()

    for t in a_scores_tasks(1, 0, 0):
        t()

    def block(j, carry):
        jp = jnp.maximum(j - 1, 0)
        mix, out = mix_tasks(jp, (j + 1) % 2, (j + 2) % 3)
        jn = jnp.minimum(j + 1, NBLK - 1)
        jn2 = jnp.minimum(j + 2, NBLK - 1)
        zero = j // NBLK
        for i in range(4):
            a_ex, a_pv = a_rest_tasks(jn, (j + 1) % 3, i, i % 2 + zero)
            if i < 3:
                a_next = a_scores_tasks(jn, i + 1, (i + 1) % 2)
            else:
                a_next = a_scores_tasks(jn2, 0, 0)
            mid = [mix] if i == 0 else []
            post = [out] if i == 3 else []
            segment(j, i, (a_ex, a_pv, a_next, mid, post))
        return carry

    jax.lax.fori_loop(0, NBLK, block, 0)

    mix, out = mix_tasks(NBLK - 1, (NBLK - 1) % 2, (NBLK - 1) % 3)
    mix()
    out()
    cp(outb.at[0], out_h.at[:, pl.ds(0, BLK)], osem).wait()


@functools.partial(jax.jit, static_argnames=("B_seg_len",))
def pallas_gated_mix__sliding_block__memory_aug_recurrent_mem_tr__prompt_kernel(A_x, A_wqkv, A_wo, B_x, B_mem0, B_Wq, B_Wk, B_Wv, B_Wo, B_seg_len, gate_w):
    assert B_seg_len == SEG
    hbm = pl.BlockSpec(memory_space=pltpu.HBM)
    scratch = [
        pltpu.VMEM((D, S), BF16),
        pltpu.VMEM((D, 3 * D), BF16),
        pltpu.VMEM((D, D), BF16),
        pltpu.VMEM((D,), BF16),
        pltpu.VMEM((S + 8, D), BF16),
        pltpu.VMEM((MEM, D), BF16),
        pltpu.VMEM((3, 2, NRC, H * RC, 128), BF16),
        pltpu.VMEM((H * D, DHB), BF16),
        pltpu.VMEM((NTILES, D // 2, 128), U32),
        pltpu.VMEM((NHT, D // 2, 128), U32),
        pltpu.VMEM((NHT, D // 2, 128), U32),
        pltpu.VMEM((NHT, D // 2, 128), U32),
        pltpu.VMEM((D, 128), F32),
        pltpu.VMEM((4, D, 128), BF16),
        pltpu.VMEM((512, D), U32),
        pltpu.VMEM((D, 512), BF16),
        pltpu.VMEM((4, S + WIN, 128), BF16),
        pltpu.VMEM((NBLK, 4, 128, 128), BF16),
        pltpu.VMEM((NBLK + 2, 4, 128, 128), BF16),
        pltpu.VMEM((NBLK, 8, 128), F32),
        pltpu.VMEM((3, 4, 128, 128), BF16),
        pltpu.VMEM((2, 4, 3 * BLK, 128), F32),
        pltpu.VMEM((2, 4, 8, BLK), F32),
        pltpu.VMEM((4, 3 * BLK, 128), BF16),
        pltpu.VMEM((NTILES, 4 * L, 128), BF16),
        pltpu.VMEM((2, 6, 48, 128), BF16),
        pltpu.VMEM((2, BLK, 512), BF16),
        pltpu.VMEM((2, D, BLK), BF16),
        pltpu.SMEM((1,), jnp.int32),
        pltpu.SemaphoreType.DMA((9,)),
        pltpu.SemaphoreType.DMA(()),
    ]
    out_t = pl.pallas_call(
        _kernel,
        out_shape=jax.ShapeDtypeStruct((D, S), BF16),
        in_specs=[hbm] * 9,
        out_specs=hbm,
        scratch_shapes=scratch,
        compiler_params=pltpu.CompilerParams(vmem_limit_bytes=100 * 1024 * 1024),
    )(
        A_x.reshape(S, D).T, A_wqkv, A_wo, B_mem0.reshape(MEM, D),
        B_Wq.reshape(D * H, DHB), B_Wk.reshape(D * H, DHB), B_Wv.reshape(D * H, DHB),
        jnp.transpose(B_Wo, (0, 2, 1)).reshape(H * D, DHB), gate_w,
    )
    return out_t.T.reshape(1, S, D)
```

```python
import functools

import jax
import jax.numpy as jnp
import jax.experimental.pallas as pl
import jax.experimental.pallas.tpu as pltpu

F32 = jnp.float32
BF16 = jnp.bfloat16
U32 = jnp.uint32

NT = (((1,), (1,)), ((), ()))

S = 2048
D = 448
H = 16
DHA = 28
DHB = 256
MEM = 8
SEG = 32
L = MEM + SEG
BLK = 128
NBLK = S // BLK
WIN = 256
NHT = H * DHB // 128
NFT = H * D // 128
NTILES = 2 * NFT
RC = 112
NRC = D // RC
NEG = -1e9
SCALE_A = 0.189453125
SCALE_B = 0.0625
GROUPS = [(0, 2, 4), (1, 3, 5), (6, 8, 10), (7, 9, 11), (12, 14), (13, 15)]


def _dot(a, b):
    return jnp.dot(a, b, preferred_element_type=F32)


def _dotg(a, b, dims):
    return jax.lax.dot_general(a, b, dims, preferred_element_type=F32)


def _kernel(xat_h, wqkv_h, woa_h, mem0_h, wq_h, wk_h, wv_h, wot_h, gate_h,
            out_h,
            xat, wqkv, woa, gate, xb, mem, raw, wot, wbig, wst, wsk, shared,
            wka, wqvt, woat, ka, qt, vt, gsig, obuf, sbuf, mxb, pbuf, xp, ptb, bbuf, outb,
            zsm, sems, osem):
    cp = pltpu.make_async_copy
    zsm[0] = 0

    def zero_like_bits(v):
        return pltpu.bitcast(v, U32) & zsm[0].astype(U32)

    c_wqkv = cp(wqkv_h, wqkv, sems.at[0])
    c_xa = cp(xat_h, xat, sems.at[1])
    c_woa = cp(woa_h, woa, sems.at[2])
    c_gate = cp(gate_h, gate, sems.at[3])
    c_mem = cp(mem0_h, mem, sems.at[4])
    c_wo = cp(wot_h, wot, sems.at[5])

    def c_w(m, src):
        return [cp(src.at[pl.ds(H * RC * r, H * RC), pl.ds(128 * c, 128)], raw.at[m, c, r], sems.at[6 + m])
                for c in range(2) for r in range(NRC)]

    c_wv, c_wq, c_wk = c_w(0, wv_h), c_w(1, wq_h), c_w(2, wk_h)
    c_wqkv.start()
    c_wqkv.wait()
    for c in [c_xa, c_gate, c_woa, c_mem]:
        c.start()

    nrow = jax.lax.broadcasted_iota(jnp.int32, (1, 128), 1)
    trow = jnp.where(nrow % 32 < DHA, DHA * (nrow // 32) + nrow % 32, -4096)
    ncol = jax.lax.broadcasted_iota(jnp.int32, (128, 1), 0)
    tcol = jnp.where(ncol % 32 < DHA, DHA * (ncol // 32) + ncol % 32, -4096)
    for p in (0, 2, 1):
        for g in range(4):
            col0 = p * D + 112 * g
            start = (col0 // 128) * 128
            width = min(256, 3 * D - start)
            win = wqkv[:, pl.ds(start, width)]
            if p == 1:
                ci = jax.lax.broadcasted_iota(jnp.int32, (width, 128), 0)
                sel = jnp.where(ci == trow + (col0 - start), 1.0, 0.0).astype(BF16)
                wka[g] = _dot(win, sel).astype(BF16)
            else:
                cit = jax.lax.broadcasted_iota(jnp.int32, (128, width), 1)
                selt = jnp.where(cit == tcol + (col0 - start), 1.0, 0.0).astype(BF16)
                row0 = (0 if p == 0 else 512) + 128 * g
                wqvt[pl.ds(row0 // 2, 64), :] = pltpu.bitcast(_dotg(selt, win, NT).astype(BF16), U32)

    lane = jax.lax.broadcasted_iota(jnp.int32, (WIN, 128), 1)
    zk = jnp.where(lane % 32 == DHA, NEG, 0.0).astype(BF16)
    for g in range(4):
        ka[g, pl.ds(0, WIN), :] = zk
    for kb in range(2):
        vt[kb] = jnp.zeros((4, 128, 128), BF16)
    c_gate.wait()
    c_woa.wait()
    cj = jax.lax.broadcasted_iota(jnp.int32, (128, 112), 1)
    selo = jnp.where(cj == tcol, 1.0, 0.0).astype(BF16)
    for g in range(4):
        wop = _dot(selo, woa[pl.ds(112 * g, 112), :]).astype(BF16)
        woat[:, pl.ds(128 * g, 128)] = wop.T

    def gated(lhs, zbits):
        if zbits is None:
            return lhs
        head = pltpu.bitcast(pltpu.bitcast(lhs[0:16, 0:128], U32) | zbits, BF16)
        top = jnp.concatenate([head, lhs[0:16, 128:]], axis=1)
        return jnp.concatenate([top, lhs[16:]], axis=0)

    def a_proj_tasks(jb):
        r0 = pl.multiple_of(jb * BLK, BLK)
        st = {}

        def tr():
            xb[pl.ds(r0, BLK), :] = xat[:, pl.ds(r0, BLK)].T

        def qv(k):
            def f(zbits):
                lhs = gated(pltpu.bitcast(wqvt[pl.ds(128 * k, 128), :], BF16), zbits)
                y = _dot(lhs, xat[:, pl.ds(r0, BLK)])
                st['last'] = y[0:1]
                st['probe'] = [y[64 * c:64 * c + 1] for c in range(4)]
                for gg in range(2):
                    g = (2 * k + gg) % 4
                    yg = y[128 * gg:128 * (gg + 1)]
                    if k < 2:
                        qpad = jax.lax.broadcasted_iota(jnp.int32, (128, BLK), 0) % 32 == DHA
                        qt[jb, g] = jnp.where(qpad, 1.0, yg * SCALE_A).astype(BF16)
                    else:
                        vt[jb + 2, g] = yg.astype(BF16)
            return f

        def kk(k):
            def f(zbits):
                if k == 0:
                    gate8 = jnp.broadcast_to(gate[...].reshape(1, D), (8, D))
                    gsig[jb] = jax.nn.sigmoid(_dot(gate8, xat[:, pl.ds(r0, BLK)]))
                xblk = gated(xb[pl.ds(r0, BLK), :], zbits)
                for g in (2 * k, 2 * k + 1):
                    y = _dot(xblk, wka[g])
                    st['last'] = y[0:1]
                    st['probe'] = [y[32 * c:32 * c + 1] for c in range(4)]
                    ka[g, pl.ds(WIN + r0, BLK), :] = y.astype(BF16)
            return f

        def gate_fn(c=None):
            v = st['last'] if c is None else st['probe'][c]
            return pltpu.bitcast(zero_like_bits(v), F32)

        return tr, [qv(0), qv(1), qv(2), qv(3), kk(0), kk(1)], gate_fn

    def a_scores_tasks(jb, g, sa):
        st = {}

        def part(kb):
            def f():
                kr = jax.lax.broadcasted_iota(jnp.int32, (BLK, BLK), 0)
                qc = jax.lax.broadcasted_iota(jnp.int32, (BLK, BLK), 1)
                kblk = ka[g, pl.ds(pl.multiple_of((jb + kb) * BLK, BLK), BLK), :]
                for hh in range(4):
                    qs = qt[jb, g, pl.ds(32 * hh, 32), :]
                    parts = []
                    if hh > 0:
                        parts.append(jnp.zeros((32 * hh, BLK), BF16))
                    parts.append(qs)
                    if hh < 3:
                        parts.append(jnp.zeros((96 - 32 * hh, BLK), BF16))
                    sk = _dot(kblk, jnp.concatenate(parts, axis=0))
                    if kb == 0:
                        sk = jnp.where(kr > qc, sk, NEG)
                    elif kb == 2:
                        sk = jnp.where(kr <= qc, sk, NEG)
                    sbuf[sa, hh, pl.ds(BLK * kb, BLK), :] = sk
                    mx = jnp.max(sk, axis=0, keepdims=True)
                    st[hh] = mx if kb == 0 else jnp.maximum(st[hh], mx)
                    if kb == 2:
                        mxb[sa, hh] = jnp.broadcast_to(st[hh], (8, BLK))
            return f
        return [part(kb) for kb in range(3)]

    def a_rest_tasks(jb, slot, g, sb):
        ch = 3 * BLK // 4
        st = {}

        def expo(hh, c):
            def f(gate_fn):
                mx = mxb[sb, hh][0:1] + gate_fn()
                e = jnp.exp(sbuf[sb, hh, pl.ds(ch * c, ch), :] - mx)
                part = jnp.sum(e, axis=0, keepdims=True)
                st[('l', hh)] = part if c == 0 else st[('l', hh)] + part
                pbuf[hh, pl.ds(ch * c, ch), :] = e.astype(BF16)
            return f

        def pv():
            for hh in range(4):
                vwin = jnp.concatenate(
                    [vt[jb + kb, g, pl.ds(32 * hh, 32), :] for kb in range(3)], axis=1)
                o = _dot(vwin, pbuf[hh]) / st[('l', hh)]
                obuf[slot, g, pl.ds(32 * hh, 32), :] = o.astype(BF16)

        return [expo(hh, c) for hh in range(4) for c in range(4)], pv

    raw32 = raw.bitcast(U32)

    def get_w(n):
        return pltpu.bitcast(wbig[n], BF16)

    def put_w(n, val):
        wbig[n] = pltpu.bitcast(val.astype(BF16), U32)

    def relay_chunk(m, dst, r, j, c, zf=None):
        a = raw32[m, c, r, pl.ds(j, RC, stride=8), :]
        if zf is not None:
            a = a | zf
        lo = pltpu.bitcast(a << 16, F32).astype(BF16)
        hi = pltpu.bitcast(a & jnp.uint32(0xFFFF0000), F32).astype(BF16)
        lo, hi = pltpu.bitcast(lo, U32), pltpu.bitcast(hi, U32)
        rows = pl.ds(pl.multiple_of(RC // 2 * r, 8), RC // 2)
        dst[4 * j + c, rows, :] = lo
        dst[4 * j + 2 + c, rows, :] = hi
        return lo[RC // 2 - 8:] | hi[RC // 2 - 8:]

    def a_proj_loop(lo, hi, relay, pre):
        def body(jb, carry):
            pre(jb)
            tr, stages, gate_fn = a_proj_tasks(jb)
            jc = [(j, c) for j in range(8) for c in range(2)]
            tr()
            due = [None] * 8
            for k, stage in enumerate(stages):
                zin = due[k]
                if k > 0:
                    chain = pltpu.bitcast(gate_fn(), U32)
                    chain = jnp.broadcast_to(chain, (8, 128))
                    zin = chain if zin is None else zin | chain
                stage(zin)
                if relay is not None and k < 4:
                    mm, dst = relay(jb)
                    z = None
                    for ci, (j, c) in enumerate(jc[4 * k:4 * k + 4]):
                        zz = relay_chunk(mm, dst, jb % NRC, j, c, pltpu.bitcast(gate_fn(ci), U32))
                        z = zz if z is None else z | zz
                    due[k + 2] = z & zsm[0].astype(U32)
            return carry
        jax.lax.fori_loop(lo, hi, body, 0)

    def starter(at, copies):
        def pre(jb):
            @pl.when(jb == at)
            def _():
                for c in copies:
                    c.start()
        return pre

    def pre2(jb):
        starter(10, c_wk)(jb)

        @pl.when(jb == 12)
        def _():
            for c in c_wq:
                c.wait()

    c_xa.wait()
    for c in c_wv:
        c.start()
    a_proj_loop(0, 8, None, starter(4, c_wq))
    c_wo.start()
    for c in c_wv:
        c.wait()
    a_proj_loop(8, 16, lambda jb: (jb // 4 - 2, wst.at[jb // 4 - 2]), pre2)

    def xrow(r):
        return (r // SEG) * L + MEM + r % SEG

    XR0 = (0, 40, 64, 104, 128)

    def main_tasks(j, i):
        nx = XR0[i + 1] - XR0[i]
        src = pl.multiple_of(j * BLK + XR0[i], 8)
        st = {}

        def prep():
            st['lhs'] = jnp.concatenate([mem[...], xb[pl.ds(src, nx), :]], axis=0)

        def tile(n):
            y32 = _dot(st['lhs'], get_w(n))
            st['last'] = y32[0:1]
            y = y32.astype(BF16)
            xp[n, pl.ds(L * i, 8), :] = y[0:8]
            for t in range(nx // 8):
                xp[n, pl.ds(xrow(XR0[i] + 8 * t), 8), :] = y[8 + 8 * t:16 + 8 * t]

        def gate_fn():
            return pltpu.bitcast(zero_like_bits(st['last']), F32)
        return prep, tile, gate_fn, (lambda: st['lhs'][0:MEM])

    c_mem.wait()
    c_wo.wait()
    z64 = jnp.zeros((64, DHB), BF16)

    def head_w(src, h):
        return jnp.concatenate([pltpu.bitcast(src[2 * h], BF16), pltpu.bitcast(src[2 * h + 1], BF16)], axis=1)

    def fold_mm(kind, j, odd, half):
        h = 2 * j + odd
        if kind == 0:
            t0, lhs, w = 7 * j, head_w(wst.at[1], h), head_w(wsk, h)
        else:
            t0, lhs, w = NFT + 7 * j, head_w(wst.at[0], h), wot[pl.ds(pl.multiple_of(D * h, 64), D), :]
        w = jnp.concatenate([z64, w] if odd else [w, z64], axis=0)[256 * half:256 * half + 256]
        b = _dotg(lhs, w, NT)
        if kind == 0:
            b = b * SCALE_B
        if not odd:
            put_w(t0 + 2 * half, b[:, 0:128])
            if half == 0:
                put_w(t0 + 1, b[:, 128:256])
            else:
                shared[...] = b[:, 128:256]
        else:
            if half == 0:
                put_w(t0 + 3, shared[...] + b[:, 0:128])
            else:
                put_w(t0 + 5, b[:, 0:128])
            put_w(t0 + 4 + 2 * half, b[:, 128:256])
        return [zero_like_bits(b[112 * c:112 * c + 1, 0:128]) for c in range(4)]

    for c in c_wk:
        c.wait()

    def u_fold(r, carry):
        kch = [(jj, c) for jj in range(8) for c in range(2)]
        nk = 0
        for jp in range(2):
            for odd in range(2):
                for half in range(2):
                    probes = fold_mm(1, 2 * r + jp, odd, half)
                    for pz in probes[1:3]:
                        relay_chunk(2, wsk, r, kch[nk][0], kch[nk][1], pz)
                        nk += 1
        return carry

    jax.lax.fori_loop(0, NRC, u_fold, 0, unroll=1)

    def t_fold(j, carry):
        for odd in range(2):
            for half in range(2):
                fold_mm(0, j, odd, half)
        return carry

    jax.lax.fori_loop(0, 8, t_fold, 0, unroll=2)

    def segment(j, i, atasks):
        st = {'acc': [None, None]}
        ptslot_w = j % 2
        ptslot_r = 1 - (j + 1) % 2
        prep, mtile, gate_fn, mem0_val = main_tasks(j, i)

        def xt(n):
            return xp[n, pl.ds(L * i, L), :]

        def window(base, h):
            return jnp.concatenate([xt(base + (7 * h) // 2 + t) for t in range(4)], axis=1)

        def b_scores(grp):
            if 'hp' not in st:
                r = pl.multiple_of((4 * j + i) * SEG, SEG)
                hrows = jnp.concatenate([mem0_val(), xb[pl.ds(r, SEG), :]], axis=0)
                z = jnp.zeros((L, 64), BF16)
                st['hp'] = [jnp.concatenate([hrows, z], axis=1), jnp.concatenate([z, hrows], axis=1)]
            t = jnp.concatenate([window(0, h) for h in grp], axis=0)
            st[grp] = _dotg(st['hp'][grp[0] % 2], t, NT)

        def b_softmax(grp):
            n = len(grp)
            row = jax.lax.broadcasted_iota(jnp.int32, (L, L * n), 0)
            lane = jax.lax.broadcasted_iota(jnp.int32, (L, L * n), 1)
            blk = [(lane >= L * a) & (lane < L * (a + 1)) for a in range(n)]
            t = lane
            for a in range(1, n):
                t = jnp.where(lane >= L * a, lane - L * a, t)
            s = jnp.where((t < MEM) | (t >= row), st[grp], NEG)
            mx = jnp.max(s, axis=0, keepdims=True)
            e = jnp.exp(s - mx)
            l = jnp.sum(e, axis=0, keepdims=True)
            p = e * (1.0 / l)
            blocks = [jnp.where(blk[a], p, 0.0) for a in range(n)]
            blocks.append(jnp.zeros((128 - L * n, L * n), F32))
            p = jnp.concatenate(blocks, axis=0)
            p = jnp.concatenate([p, jnp.zeros((128, 128 - L * n), F32)], axis=1).T
            lhs = p[0:L]
            for a in range(1, n):
                lhs = lhs + p[L * a:L * (a + 1)]
            lhs = jnp.concatenate([lhs, jnp.zeros((8, 128), F32)], axis=0)
            ptb[ptslot_w, GROUPS.index(grp)] = lhs.astype(BF16)

        def b_pv(grp):
            par = grp[0] % 2
            kk = L * len(grp)
            p = ptb[ptslot_r, GROUPS.index(grp)][:L, :kk]
            u = jnp.concatenate([window(NFT, h) for h in grp], axis=0)
            o = _dot(p, u)
            st['acc'][par] = o if st['acc'][par] is None else st['acc'][par] + o

        def fin():
            a0, a1 = st['acc']
            o = a0 + jnp.concatenate([a1[:, 64:512], jnp.zeros((L, 64), F32)], axis=1)
            ob = o.astype(BF16)
            mem[...] = ob[0:MEM, :D]
            bbuf[j % 2, pl.ds(SEG * i, SEG), :] = ob[MEM:]

        a_ex, a_pv, a_next, mid, post = atasks
        lag = 8 if i % 2 else 6
        prep()
        nex = 0
        ready_after = {g: NFT + (7 * max(g)) // 2 + 3 + lag for g in GROUPS}
        pend = list(GROUPS)
        for n in range(NTILES):
            mtile(n)
            if n >= 4 and n % 4 == 1 and nex < 16:
                a_ex[nex](gate_fn)
                nex += 1
            if n in (26, 47, 61):
                gi = {26: 0, 47: 2, 61: 4}[n]
                b_scores(GROUPS[gi])
                b_scores(GROUPS[gi + 1])
            if n in (33, 54, 68):
                b_softmax(GROUPS[{33: 0, 54: 2, 68: 4}[n]])
            if n in (38, 59, 73):
                b_softmax(GROUPS[{38: 1, 59: 3, 73: 5}[n]])
            if n == 70:
                a_pv()
            while pend and ready_after[pend[0]] <= n:
                b_pv(pend.pop(0))
        a_next[0]()
        for g in pend:
            b_pv(g)
        a_next[1]()
        for t in mid:
            t()
        a_next[2]()
        fin()
        for t in post:
            t()

    def mix_tasks(jb, slot, oslot):
        def mix():
            ot = obuf[oslot].reshape(512, BLK)
            a = _dot(woat[...], ot)
            b = bbuf[slot].T[:D].astype(F32)
            g = gsig[jb][0:1]
            outb[slot] = (g * a + (1.0 - g) * b).astype(BF16)

        def out():
            dst = out_h.at[:, pl.ds(pl.multiple_of(jb * BLK, BLK), BLK)]
            cp(outb.at[slot], dst, osem).wait()
            cp(outb.at[slot], dst, osem).start()
        return mix, out

    bbuf[1] = jnp.zeros((BLK, 512), BF16)
    obuf[1] = jnp.zeros((4, 128, BLK), BF16)
    outb[0] = jnp.zeros((D, BLK), BF16)
    cp(outb.at[0], out_h.at[:, pl.ds(0, BLK)], osem).start()

    for t in a_scores_tasks(0, 0, 0):
        t()

    def block(j, carry):
        jp = jnp.maximum(j - 1, 0)
        mix, out = mix_tasks(jp, (j + 1) % 2, (j + 1) % 2)
        jn = jnp.minimum(j + 1, NBLK - 1)
        zero = j // NBLK
        for i in range(4):
            a_ex, a_pv = a_rest_tasks(j, j % 2, i, i % 2 + zero)
            if i < 3:
                a_next = a_scores_tasks(j, i + 1, (i + 1) % 2)
            else:
                a_next = a_scores_tasks(jn, 0, 0)
            mid = [mix] if i == 0 else []
            post = [out] if i == 3 else []
            segment(j, i, (a_ex, a_pv, a_next, mid, post))
        return carry

    jax.lax.fori_loop(0, NBLK, block, 0)

    mix, out = mix_tasks(NBLK - 1, (NBLK - 1) % 2, (NBLK - 1) % 2)
    mix()
    out()
    cp(outb.at[0], out_h.at[:, pl.ds(0, BLK)], osem).wait()


@functools.partial(jax.jit, static_argnames=("B_seg_len",))
def pallas_gated_mix__sliding_block__memory_aug_recurrent_mem_tr__prompt_kernel(A_x, A_wqkv, A_wo, B_x, B_mem0, B_Wq, B_Wk, B_Wv, B_Wo, B_seg_len, gate_w):
    assert B_seg_len == SEG
    hbm = pl.BlockSpec(memory_space=pltpu.HBM)
    scratch = [
        pltpu.VMEM((D, S), BF16),
        pltpu.VMEM((D, 3 * D), BF16),
        pltpu.VMEM((D, D), BF16),
        pltpu.VMEM((D,), BF16),
        pltpu.VMEM((S + 8, D), BF16),
        pltpu.VMEM((MEM, D), BF16),
        pltpu.VMEM((3, 2, NRC, H * RC, 128), BF16),
        pltpu.VMEM((H * D, DHB), BF16),
        pltpu.VMEM((NTILES, D // 2, 128), U32),
        pltpu.VMEM((2, NHT, D // 2, 128), U32),
        pltpu.VMEM((NHT, D // 2, 128), U32),
        pltpu.VMEM((D, 128), F32),
        pltpu.VMEM((4, D, 128), BF16),
        pltpu.VMEM((512, D), U32),
        pltpu.VMEM((D, 512), BF16),
        pltpu.VMEM((4, S + WIN, 128), BF16),
        pltpu.VMEM((NBLK, 4, 128, 128), BF16),
        pltpu.VMEM((NBLK + 2, 4, 128, 128), BF16),
        pltpu.VMEM((NBLK, 8, 128), F32),
        pltpu.VMEM((2, 4, 128, 128), BF16),
        pltpu.VMEM((2, 4, 3 * BLK, 128), F32),
        pltpu.VMEM((2, 4, 8, BLK), F32),
        pltpu.VMEM((4, 3 * BLK, 128), BF16),
        pltpu.VMEM((NTILES, 4 * L, 128), BF16),
        pltpu.VMEM((2, 6, 48, 128), BF16),
        pltpu.VMEM((2, BLK, 512), BF16),
        pltpu.VMEM((2, D, BLK), BF16),
        pltpu.SMEM((1,), jnp.int32),
        pltpu.SemaphoreType.DMA((9,)),
        pltpu.SemaphoreType.DMA(()),
    ]
    out_t = pl.pallas_call(
        _kernel,
        out_shape=jax.ShapeDtypeStruct((D, S), BF16),
        in_specs=[hbm] * 9,
        out_specs=hbm,
        scratch_shapes=scratch,
        compiler_params=pltpu.CompilerParams(vmem_limit_bytes=100 * 1024 * 1024),
    )(
        A_x.reshape(S, D).T, A_wqkv, A_wo, B_mem0.reshape(MEM, D),
        B_Wq.reshape(D * H, DHB), B_Wk.reshape(D * H, DHB), B_Wv.reshape(D * H, DHB),
        jnp.transpose(B_Wo, (0, 2, 1)).reshape(H * D, DHB), gate_w,
    )
    return out_t.T.reshape(1, S, D)
```

```python
import functools

import jax
import jax.numpy as jnp
import jax.experimental.pallas as pl
import jax.experimental.pallas.tpu as pltpu

F32 = jnp.float32
BF16 = jnp.bfloat16
U32 = jnp.uint32

NT = (((1,), (1,)), ((), ()))

S = 2048
D = 448
H = 16
DHA = 28
DHB = 256
MEM = 8
SEG = 32
L = MEM + SEG
BLK = 128
NBLK = S // BLK
WIN = 256
NHT = H * DHB // 128
NFT = H * D // 128
NTILES = 2 * NFT
RC = 112
NRC = D // RC
NEG = -1e9
SCALE_A = 0.189453125
SCALE_B = 0.0625
GROUPS = [(0, 2, 4), (1, 3, 5), (6, 8, 10), (7, 9, 11), (12, 14), (13, 15)]


def _dot(a, b):
    return jnp.dot(a, b, preferred_element_type=F32)


def _dotg(a, b, dims):
    return jax.lax.dot_general(a, b, dims, preferred_element_type=F32)


def _kernel(xat_h, wqkv_h, woa_h, mem0_h, wq_h, wk_h, wv_h, wot_h, gate_h,
            out_h,
            xat, wqkv, woa, gate, xb, mem, raw, wot, wbig, wst, wsk, shared,
            wka, wqvt, woat, ka, qt, vt, gsig, obuf, sbuf, mxb, pbuf, xp, ptb, bbuf, outb,
            zsm, sems, osem):
    cp = pltpu.make_async_copy
    zsm[0] = 0

    def zero_like_bits(v):
        return pltpu.bitcast(v, U32) & zsm[0].astype(U32)

    c_wqkv = cp(wqkv_h, wqkv, sems.at[0])
    c_xa = [cp(xat_h.at[:, pl.ds(512 * c, 512)], xat.at[:, pl.ds(512 * c, 512)], sems.at[9 + c])
            for c in range(4)]
    c_woa = cp(woa_h, woa, sems.at[2])
    c_gate = cp(gate_h, gate, sems.at[3])
    c_mem = cp(mem0_h, mem, sems.at[4])
    c_wo = cp(wot_h, wot, sems.at[5])

    def c_w(m, src):
        return [cp(src.at[pl.ds(H * RC * r, H * RC), pl.ds(128 * c, 128)], raw.at[m, c, r], sems.at[6 + m])
                for c in range(2) for r in range(NRC)]

    c_wv, c_wq, c_wk = c_w(0, wv_h), c_w(1, wq_h), c_w(2, wk_h)
    c_wqkv.start()
    c_wqkv.wait()
    for c in [c_xa[0], c_gate, c_woa]:
        c.start()

    nrow = jax.lax.broadcasted_iota(jnp.int32, (1, 128), 1)
    trow = jnp.where(nrow % 32 < DHA, DHA * (nrow // 32) + nrow % 32, -4096)
    ncol = jax.lax.broadcasted_iota(jnp.int32, (128, 1), 0)
    tcol = jnp.where(ncol % 32 < DHA, DHA * (ncol // 32) + ncol % 32, -4096)
    for p in (0, 2, 1):
        if p == 2:
            for c in c_xa[1:] + [c_mem]:
                c.start()
        for g in range(4):
            col0 = p * D + 112 * g
            start = (col0 // 128) * 128
            width = min(256, 3 * D - start)
            win = wqkv[:, pl.ds(start, width)]
            if p == 1:
                ci = jax.lax.broadcasted_iota(jnp.int32, (width, 128), 0)
                sel = jnp.where(ci == trow + (col0 - start), 1.0, 0.0).astype(BF16)
                wka[g] = _dot(win, sel).astype(BF16)
            else:
                cit = jax.lax.broadcasted_iota(jnp.int32, (128, width), 1)
                selt = jnp.where(cit == tcol + (col0 - start), 1.0, 0.0).astype(BF16)
                row0 = (0 if p == 0 else 512) + 128 * g
                wqvt[pl.ds(row0 // 2, 64), :] = pltpu.bitcast(_dotg(selt, win, NT).astype(BF16), U32)

    lane = jax.lax.broadcasted_iota(jnp.int32, (WIN, 128), 1)
    zk = jnp.where(lane % 32 == DHA, NEG, 0.0).astype(BF16)
    for g in range(4):
        ka[g, pl.ds(0, WIN), :] = zk
    for kb in range(2):
        vt[kb] = jnp.zeros((4, 128, 128), BF16)
    c_gate.wait()
    c_woa.wait()
    cj = jax.lax.broadcasted_iota(jnp.int32, (128, 112), 1)
    selo = jnp.where(cj == tcol, 1.0, 0.0).astype(BF16)
    for g in range(4):
        wop = _dot(selo, woa[pl.ds(112 * g, 112), :]).astype(BF16)
        woat[:, pl.ds(128 * g, 128)] = wop.T

    def gated(lhs, zbits):
        if zbits is None:
            return lhs
        head = pltpu.bitcast(pltpu.bitcast(lhs[0:16, 0:128], U32) | zbits, BF16)
        top = jnp.concatenate([head, lhs[0:16, 128:]], axis=1)
        return jnp.concatenate([top, lhs[16:]], axis=0)

    def a_proj_tasks(jb):
        r0 = pl.multiple_of(jb * BLK, BLK)
        st = {}

        def tr():
            xb[pl.ds(r0, BLK), :] = xat[:, pl.ds(r0, BLK)].T

        def qv(k):
            def f(zbits):
                lhs = gated(pltpu.bitcast(wqvt[pl.ds(128 * k, 128), :], BF16), zbits)
                y = _dot(lhs, xat[:, pl.ds(r0, BLK)])
                st['last'] = y[0:1]
                st['probe'] = [y[64 * c:64 * c + 1] for c in range(4)]
                for gg in range(2):
                    g = (2 * k + gg) % 4
                    yg = y[128 * gg:128 * (gg + 1)]
                    if k < 2:
                        qpad = jax.lax.broadcasted_iota(jnp.int32, (128, BLK), 0) % 32 == DHA
                        qt[jb, g] = jnp.where(qpad, 1.0, yg * SCALE_A).astype(BF16)
                    else:
                        vt[jb + 2, g] = yg.astype(BF16)
            return f

        def kk(k):
            def f(zbits):
                if k == 0:
                    gate8 = jnp.broadcast_to(gate[...].reshape(1, D), (8, D))
                    gsig[jb] = jax.nn.sigmoid(_dot(gate8, xat[:, pl.ds(r0, BLK)]))
                xblk = gated(xb[pl.ds(r0, BLK), :], zbits)
                for g in (2 * k, 2 * k + 1):
                    y = _dot(xblk, wka[g])
                    st['last'] = y[0:1]
                    st['probe'] = [y[32 * c:32 * c + 1] for c in range(4)]
                    ka[g, pl.ds(WIN + r0, BLK), :] = y.astype(BF16)
            return f

        def gate_fn(c=None):
            v = st['last'] if c is None else st['probe'][c]
            return pltpu.bitcast(zero_like_bits(v), F32)

        return tr, [qv(0), qv(1), qv(2), qv(3), kk(0), kk(1)], gate_fn

    def a_scores_tasks(jb, g, sa):
        st = {}

        def part(kb):
            def f():
                kr = jax.lax.broadcasted_iota(jnp.int32, (BLK, BLK), 0)
                qc = jax.lax.broadcasted_iota(jnp.int32, (BLK, BLK), 1)
                kblk = ka[g, pl.ds(pl.multiple_of((jb + kb) * BLK, BLK), BLK), :]
                for hh in range(4):
                    qs = qt[jb, g, pl.ds(32 * hh, 32), :]
                    parts = []
                    if hh > 0:
                        parts.append(jnp.zeros((32 * hh, BLK), BF16))
                    parts.append(qs)
                    if hh < 3:
                        parts.append(jnp.zeros((96 - 32 * hh, BLK), BF16))
                    sk = _dot(kblk, jnp.concatenate(parts, axis=0))
                    if kb == 0:
                        sk = jnp.where(kr > qc, sk, NEG)
                    elif kb == 2:
                        sk = jnp.where(kr <= qc, sk, NEG)
                    sbuf[sa, hh, pl.ds(BLK * kb, BLK), :] = sk
                    mx = jnp.max(sk, axis=0, keepdims=True)
                    st[hh] = mx if kb == 0 else jnp.maximum(st[hh], mx)
                    if kb == 2:
                        mxb[sa, hh] = jnp.broadcast_to(st[hh], (8, BLK))
            return f
        return [part(kb) for kb in range(3)]

    def a_rest_tasks(jb, slot, g, sb):
        ch = 3 * BLK // 4
        st = {}

        def expo(hh, c):
            def f(gate_fn):
                mx = mxb[sb, hh][0:1] + gate_fn()
                e = jnp.exp(sbuf[sb, hh, pl.ds(ch * c, ch), :] - mx)
                part = jnp.sum(e, axis=0, keepdims=True)
                st[('l', hh)] = part if c == 0 else st[('l', hh)] + part
                pbuf[hh, pl.ds(ch * c, ch), :] = e.astype(BF16)
            return f

        def pv():
            for hh in range(4):
                vwin = jnp.concatenate(
                    [vt[jb + kb, g, pl.ds(32 * hh, 32), :] for kb in range(3)], axis=1)
                o = _dot(vwin, pbuf[hh]) / st[('l', hh)]
                obuf[slot, g, pl.ds(32 * hh, 32), :] = o.astype(BF16)

        return [expo(hh, c) for hh in range(4) for c in range(4)], pv

    raw32 = raw.bitcast(U32)

    def get_w(n):
        return pltpu.bitcast(wbig[n], BF16)

    def put_w(n, val):
        wbig[n] = pltpu.bitcast(val.astype(BF16), U32)

    def relay_chunk(m, dst, r, j, c, zf=None):
        a = raw32[m, c, r, pl.ds(j, RC, stride=8), :]
        if zf is not None:
            a = a | zf
        lo = pltpu.bitcast(a << 16, F32).astype(BF16)
        hi = pltpu.bitcast(a & jnp.uint32(0xFFFF0000), F32).astype(BF16)
        lo, hi = pltpu.bitcast(lo, U32), pltpu.bitcast(hi, U32)
        rows = pl.ds(pl.multiple_of(RC // 2 * r, 8), RC // 2)
        dst[4 * j + c, rows, :] = lo
        dst[4 * j + 2 + c, rows, :] = hi
        return lo[RC // 2 - 8:] | hi[RC // 2 - 8:]

    def a_proj_loop(lo, hi, relay, pre):
        def body(jb, carry):
            pre(jb)
            tr, stages, gate_fn = a_proj_tasks(jb)
            jc = [(j, c) for j in range(8) for c in range(2)]
            tr()
            due = [None] * 8
            for k, stage in enumerate(stages):
                zin = due[k]
                if k > 0:
                    chain = pltpu.bitcast(gate_fn(), U32)
                    chain = jnp.broadcast_to(chain, (8, 128))
                    zin = chain if zin is None else zin | chain
                stage(zin)
                if relay is not None and k < 4:
                    mm, dst = relay(jb)
                    z = None
                    for ci, (j, c) in enumerate(jc[4 * k:4 * k + 4]):
                        zz = relay_chunk(mm, dst, jb % NRC, j, c, pltpu.bitcast(gate_fn(ci), U32))
                        z = zz if z is None else z | zz
                    due[k + 2] = z & zsm[0].astype(U32)
            return carry
        jax.lax.fori_loop(lo, hi, body, 0)

    def at(jb, when, fn):
        pl.when(jb == when)(fn)

    def start_all(copies):
        return lambda: [c.start() for c in copies] and None

    def wait_all(copies):
        return lambda: [c.wait() for c in copies] and None

    def pre1(jb):
        at(jb, 4, lambda: (c_xa[1].wait(), start_all(c_wq)())[1])

    def pre2(jb):
        at(jb, 10, start_all(c_wk))
        at(jb, 12, lambda: (c_xa[3].wait(), wait_all(c_wq)())[1])

    c_xa[0].wait()
    for c in c_wv:
        c.start()
    a_proj_loop(0, 8, None, pre1)
    c_wo.start()
    c_xa[2].wait()
    for c in c_wv:
        c.wait()
    a_proj_loop(8, 16, lambda jb: (jb // 4 - 2, wst.at[jb // 4 - 2]), pre2)

    def xrow(r):
        return (r // SEG) * L + MEM + r % SEG

    XR0 = (0, 40, 64, 104, 128)

    def main_tasks(j, i):
        nx = XR0[i + 1] - XR0[i]
        src = pl.multiple_of(j * BLK + XR0[i], 8)
        st = {}

        def prep():
            st['lhs'] = jnp.concatenate([mem[...], xb[pl.ds(src, nx), :]], axis=0)

        def tile(n):
            y32 = _dot(st['lhs'], get_w(n))
            st['last'] = y32[0:1]
            y = y32.astype(BF16)
            xp[n, pl.ds(L * i, 8), :] = y[0:8]
            for t in range(nx // 8):
                xp[n, pl.ds(xrow(XR0[i] + 8 * t), 8), :] = y[8 + 8 * t:16 + 8 * t]

        def gate_fn():
            return pltpu.bitcast(zero_like_bits(st['last']), F32)
        return prep, tile, gate_fn, (lambda: st['lhs'][0:MEM])

    c_mem.wait()
    c_wo.wait()
    z64 = jnp.zeros((64, DHB), BF16)

    def head_w(src, h):
        return jnp.concatenate([pltpu.bitcast(src[2 * h], BF16), pltpu.bitcast(src[2 * h + 1], BF16)], axis=1)

    def fold_mm(kind, j, odd, half):
        h = 2 * j + odd
        if kind == 0:
            t0, lhs, w = 7 * j, head_w(wst.at[1], h), head_w(wsk, h)
        else:
            t0, lhs, w = NFT + 7 * j, head_w(wst.at[0], h), wot[pl.ds(pl.multiple_of(D * h, 64), D), :]
        w = jnp.concatenate([z64, w] if odd else [w, z64], axis=0)[256 * half:256 * half + 256]
        b = _dotg(lhs, w, NT)
        if kind == 0:
            b = b * SCALE_B
        if not odd:
            put_w(t0 + 2 * half, b[:, 0:128])
            if half == 0:
                put_w(t0 + 1, b[:, 128:256])
            else:
                shared[...] = b[:, 128:256]
        else:
            if half == 0:
                put_w(t0 + 3, shared[...] + b[:, 0:128])
            else:
                put_w(t0 + 5, b[:, 0:128])
            put_w(t0 + 4 + 2 * half, b[:, 128:256])
        return [zero_like_bits(b[112 * c:112 * c + 1, 0:128]) for c in range(4)]

    for c in c_wk:
        c.wait()

    def u_fold(r, carry):
        kch = [(jj, c) for jj in range(8) for c in range(2)]
        nk = 0
        for jp in range(2):
            for odd in range(2):
                for half in range(2):
                    probes = fold_mm(1, 2 * r + jp, odd, half)
                    for pz in probes[1:3]:
                        relay_chunk(2, wsk, r, kch[nk][0], kch[nk][1], pz)
                        nk += 1
        return carry

    jax.lax.fori_loop(0, NRC, u_fold, 0, unroll=1)

    def t_fold(j, carry):
        for odd in range(2):
            for half in range(2):
                fold_mm(0, j, odd, half)
        return carry

    jax.lax.fori_loop(0, 8, t_fold, 0, unroll=2)

    def segment(j, i, atasks):
        st = {'acc': [None, None]}
        ptslot_w = j % 2
        ptslot_r = 1 - (j + 1) % 2
        prep, mtile, gate_fn, mem0_val = main_tasks(j, i)

        def xt(n):
            return xp[n, pl.ds(L * i, L), :]

        def window(base, h):
            return jnp.concatenate([xt(base + (7 * h) // 2 + t) for t in range(4)], axis=1)

        def b_scores(grp):
            if 'hp' not in st:
                r = pl.multiple_of((4 * j + i) * SEG, SEG)
                hrows = jnp.concatenate([mem0_val(), xb[pl.ds(r, SEG), :]], axis=0)
                z = jnp.zeros((L, 64), BF16)
                st['hp'] = [jnp.concatenate([hrows, z], axis=1), jnp.concatenate([z, hrows], axis=1)]
            t = jnp.concatenate([window(0, h) for h in grp], axis=0)
            st[grp] = _dotg(st['hp'][grp[0] % 2], t, NT)

        def b_softmax(grp):
            n = len(grp)
            row = jax.lax.broadcasted_iota(jnp.int32, (L, L * n), 0)
            lane = jax.lax.broadcasted_iota(jnp.int32, (L, L * n), 1)
            blk = [(lane >= L * a) & (lane < L * (a + 1)) for a in range(n)]
            t = lane
            for a in range(1, n):
                t = jnp.where(lane >= L * a, lane - L * a, t)
            s = jnp.where((t < MEM) | (t >= row), st[grp], NEG)
            mx = jnp.max(s, axis=0, keepdims=True)
            e = jnp.exp(s - mx)
            l = jnp.sum(e, axis=0, keepdims=True)
            p = e * (1.0 / l)
            blocks = [jnp.where(blk[a], p, 0.0) for a in range(n)]
            blocks.append(jnp.zeros((128 - L * n, L * n), F32))
            p = jnp.concatenate(blocks, axis=0)
            p = jnp.concatenate([p, jnp.zeros((128, 128 - L * n), F32)], axis=1).T
            lhs = p[0:L]
            for a in range(1, n):
                lhs = lhs + p[L * a:L * (a + 1)]
            lhs = jnp.concatenate([lhs, jnp.zeros((8, 128), F32)], axis=0)
            ptb[ptslot_w, GROUPS.index(grp)] = lhs.astype(BF16)

        def b_pv(grp):
            par = grp[0] % 2
            kk = L * len(grp)
            p = ptb[ptslot_r, GROUPS.index(grp)][:L, :kk]
            u = jnp.concatenate([window(NFT, h) for h in grp], axis=0)
            o = _dot(p, u)
            st['acc'][par] = o if st['acc'][par] is None else st['acc'][par] + o

        def fin():
            a0, a1 = st['acc']
            o = a0 + jnp.concatenate([a1[:, 64:512], jnp.zeros((L, 64), F32)], axis=1)
            ob = o.astype(BF16)
            mem[...] = ob[0:MEM, :D]
            bbuf[j % 2, pl.ds(SEG * i, SEG), :] = ob[MEM:]

        a_ex, a_pv, a_next, mid, post = atasks
        lag = 8 if i % 2 else 6
        prep()
        nex = 0
        ready_after = {g: NFT + (7 * max(g)) // 2 + 3 + lag for g in GROUPS}
        pend = list(GROUPS)
        for n in range(NTILES):
            mtile(n)
            if n >= 4 and n % 4 == 1 and nex < 16:
                a_ex[nex](gate_fn)
                nex += 1
            if n in (26, 47, 61):
                gi = {26: 0, 47: 2, 61: 4}[n]
                b_scores(GROUPS[gi])
                b_scores(GROUPS[gi + 1])
            if n in (33, 54, 68):
                b_softmax(GROUPS[{33: 0, 54: 2, 68: 4}[n]])
            if n in (38, 59, 73):
                b_softmax(GROUPS[{38: 1, 59: 3, 73: 5}[n]])
            if n == 70:
                a_pv()
            while pend and ready_after[pend[0]] <= n:
                b_pv(pend.pop(0))
        a_next[0]()
        for g in pend:
            b_pv(g)
        a_next[1]()
        for t in mid:
            t()
        a_next[2]()
        fin()
        for t in post:
            t()

    def mix_tasks(jb, slot, oslot):
        def mix():
            ot = obuf[oslot].reshape(512, BLK)
            a = _dot(woat[...], ot)
            b = bbuf[slot].T[:D].astype(F32)
            g = gsig[jb][0:1]
            outb[slot] = (g * a + (1.0 - g) * b).astype(BF16)

        def out():
            dst = out_h.at[:, pl.ds(pl.multiple_of(jb * BLK, BLK), BLK)]
            cp(outb.at[slot], dst, osem).wait()
            cp(outb.at[slot], dst, osem).start()
        return mix, out

    bbuf[1] = jnp.zeros((BLK, 512), BF16)
    obuf[1] = jnp.zeros((4, 128, BLK), BF16)
    outb[0] = jnp.zeros((D, BLK), BF16)
    cp(outb.at[0], out_h.at[:, pl.ds(0, BLK)], osem).start()

    for t in a_scores_tasks(0, 0, 0):
        t()

    def block(j, carry):
        jp = jnp.maximum(j - 1, 0)
        mix, out = mix_tasks(jp, (j + 1) % 2, (j + 1) % 2)
        jn = jnp.minimum(j + 1, NBLK - 1)
        zero = j // NBLK
        for i in range(4):
            a_ex, a_pv = a_rest_tasks(j, j % 2, i, i % 2 + zero)
            if i < 3:
                a_next = a_scores_tasks(j, i + 1, (i + 1) % 2)
            else:
                a_next = a_scores_tasks(jn, 0, 0)
            mid = [mix] if i == 0 else []
            post = [out] if i == 3 else []
            segment(j, i, (a_ex, a_pv, a_next, mid, post))
        return carry

    jax.lax.fori_loop(0, NBLK, block, 0)

    mix, out = mix_tasks(NBLK - 1, (NBLK - 1) % 2, (NBLK - 1) % 2)
    mix()
    out()
    cp(outb.at[0], out_h.at[:, pl.ds(0, BLK)], osem).wait()


@functools.partial(jax.jit, static_argnames=("B_seg_len",))
def pallas_gated_mix__sliding_block__memory_aug_recurrent_mem_tr__prompt_kernel(A_x, A_wqkv, A_wo, B_x, B_mem0, B_Wq, B_Wk, B_Wv, B_Wo, B_seg_len, gate_w):
    assert B_seg_len == SEG
    hbm = pl.BlockSpec(memory_space=pltpu.HBM)
    scratch = [
        pltpu.VMEM((D, S), BF16),
        pltpu.VMEM((D, 3 * D), BF16),
        pltpu.VMEM((D, D), BF16),
        pltpu.VMEM((D,), BF16),
        pltpu.VMEM((S + 8, D), BF16),
        pltpu.VMEM((MEM, D), BF16),
        pltpu.VMEM((3, 2, NRC, H * RC, 128), BF16),
        pltpu.VMEM((H * D, DHB), BF16),
        pltpu.VMEM((NTILES, D // 2, 128), U32),
        pltpu.VMEM((2, NHT, D // 2, 128), U32),
        pltpu.VMEM((NHT, D // 2, 128), U32),
        pltpu.VMEM((D, 128), F32),
        pltpu.VMEM((4, D, 128), BF16),
        pltpu.VMEM((512, D), U32),
        pltpu.VMEM((D, 512), BF16),
        pltpu.VMEM((4, S + WIN, 128), BF16),
        pltpu.VMEM((NBLK, 4, 128, 128), BF16),
        pltpu.VMEM((NBLK + 2, 4, 128, 128), BF16),
        pltpu.VMEM((NBLK, 8, 128), F32),
        pltpu.VMEM((2, 4, 128, 128), BF16),
        pltpu.VMEM((2, 4, 3 * BLK, 128), F32),
        pltpu.VMEM((2, 4, 8, BLK), F32),
        pltpu.VMEM((4, 3 * BLK, 128), BF16),
        pltpu.VMEM((NTILES, 4 * L, 128), BF16),
        pltpu.VMEM((2, 6, 48, 128), BF16),
        pltpu.VMEM((2, BLK, 512), BF16),
        pltpu.VMEM((2, D, BLK), BF16),
        pltpu.SMEM((1,), jnp.int32),
        pltpu.SemaphoreType.DMA((13,)),
        pltpu.SemaphoreType.DMA(()),
    ]
    out_t = pl.pallas_call(
        _kernel,
        out_shape=jax.ShapeDtypeStruct((D, S), BF16),
        in_specs=[hbm] * 9,
        out_specs=hbm,
        scratch_shapes=scratch,
        compiler_params=pltpu.CompilerParams(vmem_limit_bytes=100 * 1024 * 1024),
    )(
        A_x.reshape(S, D).T, A_wqkv, A_wo, B_mem0.reshape(MEM, D),
        B_Wq.reshape(D * H, DHB), B_Wk.reshape(D * H, DHB), B_Wv.reshape(D * H, DHB),
        jnp.transpose(B_Wo, (0, 2, 1)).reshape(H * D, DHB), gate_w,
    )
    return out_t.T.reshape(1, S, D)
```
